```python
import jax
import jax.numpy as jnp

def _softmax(x, axis=-1):
    return jax.nn.softmax(x, axis=axis)

def _gelu(x):
    return jax.nn.gelu(x, approximate=True)

def _silu(x):
    return jax.nn.silu(x)

def _sigmoid(x):
    return jax.nn.sigmoid(x)

def _layernorm(x, axis=-1, eps=1e-05):
    m = jnp.mean(x, axis=axis, keepdims=True)
    v = jnp.var(x, axis=axis, keepdims=True)
    return (x - m) / jnp.sqrt(v + eps)

def _scatter_add(tgt, idx, src, axis=0):
    return tgt.at[idx].add(src)

def _segment_sum(src, seg, n):
    return jax.ops.segment_sum(src, seg, n)

class _Rng:

    def __init__(self, key):
        self._k = key

    def _next(self):
        self._k, sub = jax.random.split(self._k)
        return sub

    def normal(self, shape):
        return jax.random.normal(self._next(), shape, dtype=jnp.bfloat16)

    def randint(self, lo, hi, shape):
        return jax.random.randint(self._next(), shape, lo, hi, dtype=jnp.int32)

    def uniform(self, shape, lo=0.0, hi=1.0):
        return jax.random.uniform(self._next(), shape, jnp.bfloat16, lo, hi)

    def permutation(self, n):
        return jax.random.permutation(self._next(), n)
kernel_name = 'adaLN_cond__sliding_local_dilated__swiglu_ffn__prompt'

def setup_inputs():
    _rng = _Rng(jax.random.key(int.from_bytes(__import__("os").urandom(4), "little")))
    _w = lambda a: (lambda t: t.astype(jnp.bfloat16) if jnp.issubdtype(t.dtype, jnp.floating) else t)(jnp.asarray(a))

    def _A_setup():
        B, S, D = (1, 2048, 1024)
        return {'x': _w((lambda *s: _rng.normal(s) * 0.05)(B, S, D)), 'wqkv': _w((lambda *s: _rng.normal(s) * 0.05)(D, 3 * D)), 'wo': _w((lambda *s: _rng.normal(s) * 0.05)(D, D))}
    _A_in = _A_setup()

    def _B_setup():
        B, S, D, F = (1, 2048, 1024, 3584)
        return {'x': _w((lambda *s: _rng.normal(s) * 0.05)(B, S, D)), 'w_gate': _w((lambda *s: _rng.normal(s) * 0.05)(D, F)), 'w_up': _w((lambda *s: _rng.normal(s) * 0.05)(D, F)), 'w_down': _w((lambda *s: _rng.normal(s) * 0.05)(F, D))}
    _B_in = _B_setup()
    return {'A_x': _A_in['x'], 'A_wqkv': _A_in['wqkv'], 'A_wo': _A_in['wo'], 'B_x': _B_in['x'], 'B_w_gate': _B_in['w_gate'], 'B_w_up': _B_in['w_up'], 'B_w_down': _B_in['w_down'], 'c': _w((lambda *s: _rng.normal(s) * 0.05)(1, 1024)), 'w_mod': _w((lambda *s: _rng.normal(s) * 0.05)(1024, 6 * 1024) * 1024 ** (-0.5))}

def reference(A_x, A_wqkv, A_wo, B_x, B_w_gate, B_w_up, B_w_down, c, w_mod):

    def _A_ref(x, wqkv, wo):
        B, S, D = x.shape
        H = 32
        Dh = D // H
        W, dil = (8, 2)
        qkv = (lambda x, *d: x.transpose(*d))((x @ wqkv).reshape(B, S, 3, H, Dh), 2, 0, 3, 1, 4)
        q, k, v = (qkv[0], qkv[1], qkv[2])
        scale = Dh ** (-0.5)
        pos = jnp.arange(S)
        off = jnp.arange(W) * dil
        idx = pos[:, None] - off[None, :]
        mask = idx >= 0
        idx_c = jnp.where(mask, idx, 0).reshape(-1)
        kg = k[:, :, idx_c, :].reshape(B, H, S, W, Dh)
        vg = v[:, :, idx_c, :].reshape(B, H, S, W, Dh)
        logits = jnp.einsum('bhsd,bhswd->bhsw', q, kg) * scale
        logits = jnp.where(mask[None, None, :, :], logits, -1000000000.0)
        attn = _softmax(logits, axis=-1)
        o = jnp.einsum('bhsw,bhswd->bhsd', attn, vg)
        return (lambda x, *d: x.transpose(*d))(o, 0, 2, 1, 3).reshape(B, S, D) @ wo

    def _B_ref(x, w_gate, w_up, w_down):
        g = _silu(x @ w_gate)
        u = x @ w_up
        return g * u @ w_down
    x = A_x
    mod = (_silu(c) @ w_mod).reshape(c.shape[0], 6, 1, -1)
    sa, ca, ga, sb, cb, gb = (mod[:, 0].copy(), mod[:, 1].copy(), mod[:, 2].copy(), mod[:, 3].copy(), mod[:, 4].copy(), mod[:, 5].copy())
    h = _layernorm(x, axis=-1) * (1 + ca) + sa
    x = x + ga * _A_ref(h, A_wqkv, A_wo)
    h = _layernorm(x, axis=-1) * (1 + cb) + sb
    x = x + gb * _B_ref(h, B_w_gate, B_w_up, B_w_down)
    return x
```

```python
import jax
import jax.numpy as jnp
from jax import lax
from jax.experimental import pallas as pl
from jax.experimental.pallas import tpu as pltpu

S, D, F = 2048, 1024, 3584
H, DH, W, DIL = 32, 32, 8, 2
LANES = 128
NT = D // LANES
HALO = 16
TA = 256
RB = 32
TC = 512
FC = 512
EPS = 1e-5
F32, BF16 = jnp.float32, jnp.bfloat16


def _layernorm(x):
    m = jnp.mean(x, axis=-1, keepdims=True)
    xc = x - m
    v = jnp.mean(xc * xc, axis=-1, keepdims=True)
    return xc * lax.rsqrt(v + EPS)


def _silu(x):
    return x * (1.0 / (1.0 + jnp.exp(-x)))


def _kernel(x_hbm, wqkv_hbm, wo_hbm, wg_hbm, wu_hbm, wd_hbm, c_ref, wmod_hbm, out_hbm,
            x_v, wqkv_v, wo_raw, wo_v, wg_v, wu_v, wd_v, wmod_v, mod_v,
            q_v, k_v, v_v, o_v, act_v, out_v, sems, out_sems):
    def col_copy(src, dst, lo, n, sem):
        return pltpu.make_async_copy(src.at[:, pl.ds(lo, n)], dst.at[:, pl.ds(lo, n)], sems.at[sem])

    cp_mod_a = col_copy(wmod_hbm, wmod_v, 0, 2 * D, 0)
    cp_x0 = pltpu.make_async_copy(x_hbm.at[pl.ds(0, TA)], x_v.at[pl.ds(0, TA)], sems.at[1])
    cp_qkv = [col_copy(wqkv_hbm, wqkv_v, p * D, D, 2 + p) for p in range(3)]
    cp_x1 = pltpu.make_async_copy(x_hbm.at[pl.ds(TA, S - TA)], x_v.at[pl.ds(TA, S - TA)], sems.at[5])
    cp_mod_b = col_copy(wmod_hbm, wmod_v, 2 * D, 4 * D, 6)
    cp_wo = pltpu.make_async_copy(wo_hbm, wo_raw, sems.at[7])
    cp_wg = pltpu.make_async_copy(wg_hbm, wg_v, sems.at[8])
    cp_wu = pltpu.make_async_copy(wu_hbm, wu_v, sems.at[9])
    cp_wd = pltpu.make_async_copy(wd_hbm, wd_v, sems.at[10])
    for cp in (cp_mod_a, cp_x0, *cp_qkv, cp_x1, cp_mod_b, cp_wo, cp_wg, cp_wu, cp_wd):
        cp.start()

    sc = _silu(c_ref[...].astype(F32)).astype(BF16)
    sc = jnp.broadcast_to(sc, (16, D))

    def mod_part(lo, n):
        r = jnp.dot(sc, wmod_v[:, lo:lo + n], preferred_element_type=F32)
        mod_v[:, lo:lo + n] = r[0:8].astype(BF16).astype(F32)

    def mod_row(i):
        return mod_v[0:1, i * D:(i + 1) * D]

    cp_mod_a.wait()
    mod_part(0, 2 * D)

    PR = 64
    lane_p = lax.broadcasted_iota(jnp.int32, (PR // 2, LANES), 1)

    def permute_cols(p):
        def body(r, carry):
            rows = pl.ds(pl.multiple_of(r * PR, PR), PR)
            t = [pltpu.bitcast(wqkv_v[rows, p * D + j * LANES:p * D + (j + 1) * LANES], jnp.uint32)
                 for j in range(NT)]
            for b in range(3):
                sh = 4 << b
                low = (lane_p & sh) == 0
                for j in range(NT):
                    if j & (1 << b):
                        continue
                    lo_t, hi_t = t[j], t[j | (1 << b)]
                    t[j] = jnp.where(low, lo_t, pltpu.roll(hi_t, sh, 1))
                    t[j | (1 << b)] = jnp.where(low, pltpu.roll(lo_t, LANES - sh, 1), hi_t)
            for j in range(NT):
                wqkv_v[rows, p * D + j * LANES:p * D + (j + 1) * LANES] = pltpu.bitcast(t[j], BF16)
            return carry
        lax.fori_loop(0, D // PR, body, 0)

    for p in range(3):
        cp_qkv[p].wait()
        permute_cols(p)

    def qkv_tile(r0):
        rows = pl.ds(r0, TA)
        h = _layernorm(x_v[rows, :].astype(F32)) * (1.0 + mod_row(1)) + mod_row(0)
        h = h.astype(BF16)
        q_v[rows, :] = jnp.dot(h, wqkv_v[:, 0:D], preferred_element_type=F32)
        krows = pl.ds(r0 + HALO, TA)
        k_v[krows, :] = jnp.dot(h, wqkv_v[:, D:2 * D], preferred_element_type=F32)
        v_v[krows, :] = jnp.dot(h, wqkv_v[:, 2 * D:3 * D], preferred_element_type=F32)

    lane_a = lax.broadcasted_iota(jnp.int32, (RB, LANES), 1)
    row_a = lax.broadcasted_iota(jnp.int32, (RB, LANES), 0)
    even1 = (lane_a & 1) == 0
    even2 = (lane_a & 2) == 0
    scale = DH ** -0.5

    def shifted(ref, r0, i):
        win = ref[pl.ds(r0, RB + HALO), i * LANES:(i + 1) * LANES]
        out = [None] * W
        for c in range(W // 2):
            lo = HALO - 8 - DIL * c
            blk = win[lo:lo + RB + 8]
            out[c] = blk[8:]
            out[c + W // 2] = blk[:RB]
        return out

    def attn_block(r0):
        logit = [None] * W
        for i in range(NT):
            qi = q_v[pl.ds(r0, RB), i * LANES:(i + 1) * LANES]
            ks = shifted(k_v, r0, i)
            for w in range(W):
                pr = qi * ks[w]
                logit[w] = pr if i == 0 else logit[w] + pr
        pos = row_a + r0
        for w in range(W):
            s = logit[w]
            s = s + jnp.where(even1, pltpu.roll(s, LANES - 1, 1), pltpu.roll(s, 1, 1))
            s = s + jnp.where(even2, pltpu.roll(s, LANES - 2, 1), pltpu.roll(s, 2, 1))
            s = s * scale
            logit[w] = s if w == 0 else jnp.where(pos >= DIL * w, s, -1e9)
        m = logit[0]
        for w in range(1, W):
            m = jnp.maximum(m, logit[w])
        e = [jnp.exp(s - m) for s in logit]
        den = e[0]
        for w in range(1, W):
            den = den + e[w]
        inv = 1.0 / den
        prob = [ew * inv for ew in e]
        for i in range(NT):
            vs = shifted(v_v, r0, i)
            acc = prob[0] * vs[0]
            for w in range(1, W):
                acc = acc + prob[w] * vs[w]
            o_v[pl.ds(r0, RB), i * LANES:(i + 1) * LANES] = acc.astype(BF16)

    def attn_tile(r0):
        for b in range(TA // RB):
            attn_block(pl.multiple_of(r0 + b * RB, RB))

    cp_x0.wait()
    qkv_tile(0)
    k_v[0:HALO, :] = jnp.broadcast_to(k_v[HALO:HALO + 1, :], (HALO, D))
    v_v[0:HALO, :] = jnp.broadcast_to(v_v[HALO:HALO + 1, :], (HALO, D))
    cp_x1.wait()

    def phase_a(s, carry):
        r0 = pl.multiple_of(s * TA, TA)
        attn_tile(r0 - TA)
        qkv_tile(r0)
        return carry
    lax.fori_loop(1, S // TA, phase_a, 0)

    def last_attn(b, carry):
        attn_block(pl.multiple_of(S - TA + b * RB, RB))
        return carry
    lax.fori_loop(0, TA // RB, last_attn, 0)

    cp_mod_b.wait()
    mod_part(2 * D, 4 * D)
    cp_wo.wait()
    for i in range(NT):
        for jp in range(NT // 2):
            for hh in range(4):
                pieces = []
                for j in (2 * jp, 2 * jp + 1):
                    src = (4 * j + hh) * DH + 4 * i
                    grp = wo_raw[src // 16 * 16:src // 16 * 16 + 16, :].astype(F32)
                    pieces.append(grp[src % 16:src % 16 + 4])
                dst = i * LANES + hh * DH + jp * 8
                wo_v[dst:dst + 8, :] = jnp.concatenate(pieces, axis=0)
    cp_wg.wait()
    cp_wu.wait()
    cp_wd.wait()

    def out_copy(t, slot):
        return pltpu.make_async_copy(out_v.at[slot], out_hbm.at[pl.ds(t * TC, TC)], out_sems.at[slot])

    def phase_c(t, carry):
        rows = pl.ds(pl.multiple_of(t * TC, TC), TC)
        slot = t % 2
        a = jnp.dot(o_v[rows, :], wo_v[...].astype(BF16), preferred_element_type=F32)
        x1 = x_v[rows, :].astype(F32) + mod_row(2) * a
        h = (_layernorm(x1) * (1.0 + mod_row(4)) + mod_row(3)).astype(BF16)
        for f in range(F // FC):
            cols = slice(f * FC, (f + 1) * FC)
            g = jnp.dot(h, wg_v[:, cols], preferred_element_type=F32)
            u = jnp.dot(h, wu_v[:, cols], preferred_element_type=F32)
            act_v[:, cols] = (_silu(g) * u).astype(BF16)
        y = jnp.dot(act_v[...], wd_v[...], preferred_element_type=F32)

        @pl.when(t >= 2)
        def _():
            out_copy(t - 2, slot).wait()
        out_v[slot] = (x1 + mod_row(5) * y).astype(BF16)
        out_copy(t, slot).start()
        return carry
    n_c = S // TC
    lax.fori_loop(0, n_c, phase_c, 0)
    for t in range(n_c - 2, n_c):
        out_copy(t, t % 2).wait()


@jax.jit
def pallas_adaLN_cond__sliding_local_dilated__swiglu_ffn__prompt_kernel(
    A_x: jax.Array,
    A_wqkv: jax.Array,
    A_wo: jax.Array,
    B_x: jax.Array,
    B_w_gate: jax.Array,
    B_w_up: jax.Array,
    B_w_down: jax.Array,
    c: jax.Array,
    w_mod: jax.Array,
):
    del B_x
    hbm = pl.BlockSpec(memory_space=pl.ANY)
    out = pl.pallas_call(
        _kernel,
        out_shape=jax.ShapeDtypeStruct((S, D), BF16),
        in_specs=[hbm, hbm, hbm, hbm, hbm, hbm, pl.BlockSpec(memory_space=pltpu.VMEM), hbm],
        out_specs=hbm,
        scratch_shapes=[
            pltpu.VMEM((S, D), BF16),
            pltpu.VMEM((D, 3 * D), BF16),
            pltpu.VMEM((D, D), BF16),
            pltpu.VMEM((D, D), F32),
            pltpu.VMEM((D, F), BF16),
            pltpu.VMEM((D, F), BF16),
            pltpu.VMEM((F, D), BF16),
            pltpu.VMEM((D, 6 * D), BF16),
            pltpu.VMEM((8, 6 * D), F32),
            pltpu.VMEM((S, D), F32),
            pltpu.VMEM((S + HALO, D), F32),
            pltpu.VMEM((S + HALO, D), F32),
            pltpu.VMEM((S, D), BF16),
            pltpu.VMEM((TC, F), BF16),
            pltpu.VMEM((2, TC, D), BF16),
            pltpu.SemaphoreType.DMA((11,)),
            pltpu.SemaphoreType.DMA((2,)),
        ],
        compiler_params=pltpu.CompilerParams(vmem_limit_bytes=120 * 1024 * 1024),
    )(A_x.reshape(S, D), A_wqkv, A_wo, B_w_gate, B_w_up, B_w_down, c, w_mod)
    return out.reshape(1, S, D)
```

```python
import jax
import jax.numpy as jnp
from jax import lax
from jax.experimental import pallas as pl
from jax.experimental.pallas import tpu as pltpu

S, D, F = 2048, 1024, 3584
H, DH, W, DIL = 32, 32, 8, 2
LANES = 128
NT = D // LANES
HALO = 16
TA = 256
RB = 32
TC = 512
NP, KP = 128, 512
EPS = 1e-5
F32, BF16 = jnp.float32, jnp.bfloat16


def _layernorm(x):
    m = jnp.mean(x, axis=-1, keepdims=True)
    xc = x - m
    v = jnp.mean(xc * xc, axis=-1, keepdims=True)
    return xc * lax.rsqrt(v + EPS)


def _silu(x):
    return x * (1.0 / (1.0 + jnp.exp(-x)))


ATTN_STAGES = W // 2 + 1 + NT


class _Spread:
    def __init__(self, gen, n_stages, n_slots, never):
        self.gen, self.n_stages, self.n_slots, self.never = gen, n_stages, n_slots, never
        self.slot = self.done = 0
        self.pending = []

    def step(self, part):
        if self.pending:
            n = len(self.pending) * RB
            head = jnp.where(self.never, jnp.concatenate(self.pending, axis=0), part[:n])
            part = jnp.concatenate([head, part[n:]], axis=0)
        self.pending = []
        self.slot += 1
        while self.done < min(self.n_stages, self.n_stages * self.slot // (self.n_slots - 1)):
            self.pending += next(self.gen)
            self.done += 1
        return part


def _kernel(x_hbm, wqkv_hbm, wo_hbm, wg_hbm, wu_hbm, wd_hbm, c_ref, wmod_hbm, out_hbm,
            x_v, wqkv_v, wo_raw, wo_v, wg_v, wu_v, wd_v, wmod_v, mod_v,
            q_v, k_v, v_v, o_v, act_v, h_v, x1_v, accg_v, accu_v, out_v, sems, out_sems):
    def col_copy(src, dst, lo, n, sem):
        return pltpu.make_async_copy(src.at[:, pl.ds(lo, n)], dst.at[:, pl.ds(lo, n)], sems.at[sem])

    cp_mod_a = col_copy(wmod_hbm, wmod_v, 0, 2 * D, 0)
    cp_x0 = pltpu.make_async_copy(x_hbm.at[pl.ds(0, TA)], x_v.at[pl.ds(0, TA)], sems.at[1])
    cp_qkv = [col_copy(wqkv_hbm, wqkv_v, p * D, D, 2 + p) for p in range(3)]
    cp_x1 = pltpu.make_async_copy(x_hbm.at[pl.ds(TA, S - TA)], x_v.at[pl.ds(TA, S - TA)], sems.at[5])
    cp_mod_b = col_copy(wmod_hbm, wmod_v, 2 * D, 4 * D, 6)
    cp_wo = pltpu.make_async_copy(wo_hbm, wo_raw, sems.at[7])
    cp_wg = pltpu.make_async_copy(wg_hbm, wg_v, sems.at[8])
    cp_wu = pltpu.make_async_copy(wu_hbm, wu_v, sems.at[9])
    cp_wd = pltpu.make_async_copy(wd_hbm, wd_v, sems.at[10])
    for cp in (cp_mod_a, cp_x0, cp_qkv[0]):
        cp.start()

    sc = _silu(c_ref[...].astype(F32)).astype(BF16)
    sc = jnp.broadcast_to(sc, (16, D))

    def mod_part(lo, n):
        r = jnp.dot(sc, wmod_v[:, lo:lo + n], preferred_element_type=F32)
        mod_v[:, lo:lo + n] = r[0:8].astype(BF16).astype(F32)

    def mod_row(i):
        return mod_v[0:1, i * D:(i + 1) * D]

    cp_mod_a.wait()
    cp_qkv[1].start()
    mod_part(0, 2 * D)

    PR = 128
    lane_p = lax.broadcasted_iota(jnp.int32, (PR // 2, LANES), 1)

    def permute_cols(p):
        def body(r, carry):
            rows = pl.ds(pl.multiple_of(r * PR, PR), PR)
            t = [pltpu.bitcast(wqkv_v[rows, p * D + j * LANES:p * D + (j + 1) * LANES], jnp.uint32)
                 for j in range(NT)]
            for b in range(3):
                sh = 4 << b
                low = (lane_p & sh) == 0
                for j in range(NT):
                    if j & (1 << b):
                        continue
                    lo_t, hi_t = t[j], t[j | (1 << b)]
                    t[j] = jnp.where(low, lo_t, pltpu.roll(hi_t, sh, 1))
                    t[j | (1 << b)] = jnp.where(low, pltpu.roll(lo_t, LANES - sh, 1), hi_t)
            for j in range(NT):
                wqkv_v[rows, p * D + j * LANES:p * D + (j + 1) * LANES] = pltpu.bitcast(t[j], BF16)
            return carry
        lax.fori_loop(0, D // PR, body, 0)

    def mod_ln_a(r0):
        h = _layernorm(x_v[pl.ds(r0, TA), :].astype(F32)) * (1.0 + mod_row(1)) + mod_row(0)
        return h.astype(BF16)

    def matmul_piece(lhs_ref, w_ref, lo, acc_ref, side):
        n_k = w_ref.shape[0] // KP
        for i in range(n_k):
            part = jnp.dot(lhs_ref[:, i * KP:(i + 1) * KP], w_ref[i * KP:(i + 1) * KP, lo:lo + NP].astype(BF16),
                           preferred_element_type=F32)
            if i > 0:
                part = acc_ref[...] + part
            if side is not None:
                part = side.step(part)
            if i == n_k - 1:
                return part
            acc_ref[...] = part

    def project(p, r0, side=None):
        dst, off = ((q_v, 0), (k_v, HALO), (v_v, HALO))[p]
        for n, lo in enumerate(range(0, D, NP)):
            acc = (accg_v, accu_v)[n % 2].at[0:TA]
            dst[pl.ds(r0 + off, TA), lo:lo + NP] = matmul_piece(h_v.at[0:TA], wqkv_v, p * D + lo, acc, side)

    lane_a = lax.broadcasted_iota(jnp.int32, (RB, LANES), 1)
    row_a = lax.broadcasted_iota(jnp.int32, (RB, LANES), 0)
    even1 = (lane_a & 1) == 0
    even2 = (lane_a & 2) == 0
    scale = DH ** -0.5

    def shifted(ref, r0, i, c):
        win = ref[pl.ds(r0, RB + HALO), i * LANES:(i + 1) * LANES]
        lo = HALO - 8 - DIL * c
        blk = win[lo:lo + RB + 8]
        return blk[8:], blk[:RB]

    def attn_block(r0):
        logit = [None] * W
        pos = row_a + r0
        for c in range(W // 2):
            ws = (c, c + W // 2)
            for i in range(NT):
                qi = q_v[pl.ds(r0, RB), i * LANES:(i + 1) * LANES]
                for w, kw in zip(ws, shifted(k_v, r0, i, c)):
                    logit[w] = qi * kw if i == 0 else logit[w] + qi * kw
            for w in ws:
                s = logit[w]
                s = s + jnp.where(even1, pltpu.roll(s, LANES - 1, 1), pltpu.roll(s, 1, 1))
                s = s + jnp.where(even2, pltpu.roll(s, LANES - 2, 1), pltpu.roll(s, 2, 1))
                s = s * scale
                logit[w] = s if w == 0 else jnp.where(pos >= DIL * w, s, -1e9)
            yield [logit[w] for w in ws]
        m = logit[0]
        for w in range(1, W):
            m = jnp.maximum(m, logit[w])
        e = [jnp.exp(s - m) for s in logit]
        den = e[0]
        for w in range(1, W):
            den = den + e[w]
        inv = 1.0 / den
        prob = [ew * inv for ew in e]
        yield [inv]
        for i in range(NT):
            acc = None
            for c in range(W // 2):
                for w, vw in zip((c, c + W // 2), shifted(v_v, r0, i, c)):
                    acc = prob[w] * vw if acc is None else acc + prob[w] * vw
            o_v[pl.ds(r0, RB), i * LANES:(i + 1) * LANES] = acc.astype(BF16)
            yield [acc]

    def never(r0):
        return lax.broadcasted_iota(jnp.int32, (1, LANES), 1) + r0 < 0

    def attn_rows(r0, n_blocks):
        for b in range(n_blocks):
            yield from attn_block(pl.multiple_of(r0 + b * RB, RB))

    cp_x0.wait()
    h_v[0:TA, :] = mod_ln_a(0)
    cp_qkv[0].wait()
    cp_qkv[2].start()
    cp_x1.start()
    permute_cols(0)
    project(0, 0)
    cp_qkv[1].wait()
    for cp in (cp_mod_b, cp_wo, cp_wg, cp_wu, cp_wd):
        cp.start()
    permute_cols(1)
    project(1, 0)
    cp_qkv[2].wait()
    permute_cols(2)
    project(2, 0)
    k_v[0:HALO, :] = jnp.broadcast_to(k_v[HALO:HALO + 1, :], (HALO, D))
    v_v[0:HALO, :] = jnp.broadcast_to(v_v[HALO:HALO + 1, :], (HALO, D))
    cp_x1.wait()

    n_a = S // TA
    per_a = -(-(TC // RB) // (n_a - 1))

    def phase_a(s, h):
        r0 = pl.multiple_of(s * TA, TA)
        h_v[0:TA, :] = h
        side = _Spread(attn_rows((s - 1) * per_a * RB, per_a), per_a * ATTN_STAGES, 3 * D // NP * (D // KP), never(r0))
        for p in range(3):
            project(p, r0, side)
        return mod_ln_a(pl.multiple_of(jnp.minimum(s + 1, n_a - 1) * TA, TA))
    lax.fori_loop(1, n_a, phase_a, mod_ln_a(TA))

    cp_mod_b.wait()
    mod_part(2 * D, 4 * D)
    cp_wo.wait()
    for i in range(NT):
        for jp in range(NT // 2):
            for hh in range(4):
                pieces = []
                for j in (2 * jp, 2 * jp + 1):
                    src = (4 * j + hh) * DH + 4 * i
                    grp = wo_raw[src // 16 * 16:src // 16 * 16 + 16, :].astype(F32)
                    pieces.append(grp[src % 16:src % 16 + 4])
                dst = i * LANES + hh * DH + jp * 8
                wo_v[dst:dst + 8, :] = jnp.concatenate(pieces, axis=0)
    cp_wg.wait()
    cp_wu.wait()
    cp_wd.wait()

    def out_copy(t, slot):
        return pltpu.make_async_copy(out_v.at[slot], out_hbm.at[pl.ds(t * TC, TC)], out_sems.at[slot])

    n_c = S // TC

    def phase_c(t, carry):
        rows = pl.ds(pl.multiple_of(t * TC, TC), TC)
        slot = t % 2

        @pl.when(t >= 2)
        def _():
            out_copy(t - 2, slot).wait()
        for n, lo in enumerate(range(0, D, NP)):
            a = matmul_piece(o_v.at[rows], wo_v, lo, (accg_v, accu_v)[n % 2], None)
            x1_v[:, lo:lo + NP] = x_v[rows, lo:lo + NP].astype(F32) + mod_row(2)[:, lo:lo + NP] * a
        h_v[0:TC, :] = (_layernorm(x1_v[...]) * (1.0 + mod_row(4)) + mod_row(3)).astype(BF16)
        nxt = jnp.minimum(t + 1, n_c - 1) * TC
        n_slots = 3 * (F // NP) * (D // KP)
        side = _Spread(attn_rows(nxt, TC // RB), TC // RB * ATTN_STAGES, n_slots, never(nxt))
        for lo in range(0, F, NP):
            accg_v[...] = matmul_piece(h_v.at[0:TC], wg_v, lo, accg_v, side)
            u = matmul_piece(h_v.at[0:TC], wu_v, lo, accu_v, side)
            act_v[:, lo:lo + NP] = (_silu(accg_v[...]) * u).astype(BF16)
        for n, lo in enumerate(range(0, D, NP)):
            y = matmul_piece(act_v, wd_v, lo, (accg_v, accu_v)[n % 2], side)
            out_v[slot, :, lo:lo + NP] = (x1_v[:, lo:lo + NP] + mod_row(5)[:, lo:lo + NP] * y).astype(BF16)
        out_copy(t, slot).start()
        return carry
    lax.fori_loop(0, n_c, phase_c, 0)
    for t in range(n_c - 2, n_c):
        out_copy(t, t % 2).wait()


@jax.jit
def pallas_adaLN_cond__sliding_local_dilated__swiglu_ffn__prompt_kernel(
    A_x: jax.Array,
    A_wqkv: jax.Array,
    A_wo: jax.Array,
    B_x: jax.Array,
    B_w_gate: jax.Array,
    B_w_up: jax.Array,
    B_w_down: jax.Array,
    c: jax.Array,
    w_mod: jax.Array,
):
    del B_x
    hbm = pl.BlockSpec(memory_space=pl.ANY)
    out = pl.pallas_call(
        _kernel,
        out_shape=jax.ShapeDtypeStruct((S, D), BF16),
        in_specs=[hbm, hbm, hbm, hbm, hbm, hbm, pl.BlockSpec(memory_space=pltpu.VMEM), hbm],
        out_specs=hbm,
        scratch_shapes=[
            pltpu.VMEM((S, D), BF16),
            pltpu.VMEM((D, 3 * D), BF16),
            pltpu.VMEM((D, D), BF16),
            pltpu.VMEM((D, D), F32),
            pltpu.VMEM((D, F), BF16),
            pltpu.VMEM((D, F), BF16),
            pltpu.VMEM((F, D), BF16),
            pltpu.VMEM((D, 6 * D), BF16),
            pltpu.VMEM((8, 6 * D), F32),
            pltpu.VMEM((S, D), F32),
            pltpu.VMEM((S + HALO, D), F32),
            pltpu.VMEM((S + HALO, D), F32),
            pltpu.VMEM((S, D), BF16),
            pltpu.VMEM((TC, F), BF16),
            pltpu.VMEM((max(TA, TC), D), BF16),
            pltpu.VMEM((TC, D), F32),
            pltpu.VMEM((TC, NP), F32),
            pltpu.VMEM((TC, NP), F32),
            pltpu.VMEM((2, TC, D), BF16),
            pltpu.SemaphoreType.DMA((11,)),
            pltpu.SemaphoreType.DMA((2,)),
        ],
        compiler_params=pltpu.CompilerParams(vmem_limit_bytes=120 * 1024 * 1024),
    )(A_x.reshape(S, D), A_wqkv, A_wo, B_w_gate, B_w_up, B_w_down, c, w_mod)
    return out.reshape(1, S, D)
```

```python
import jax
import jax.numpy as jnp
from jax import lax
from jax.experimental import pallas as pl
from jax.experimental.pallas import tpu as pltpu

S, D, F = 2048, 1024, 3584
H, DH, W, DIL = 32, 32, 8, 2
LANES = 128
NT = D // LANES
HALO = 16
TA = 512
RB = 32
TC = 512
NP, KP = 128, 512
PR = 64
LB = 32
MOD_ROWS, MA, MB = 16, 256, 32
EPS = 1e-5
F32, BF16, U32 = jnp.float32, jnp.bfloat16, jnp.uint32


def _layernorm(x):
    m = jnp.mean(x, axis=-1, keepdims=True)
    xc = x - m
    v = jnp.mean(xc * xc, axis=-1, keepdims=True)
    return xc * lax.rsqrt(v + EPS)


def _silu(x):
    return x * (1.0 / (1.0 + jnp.exp(-x)))


ATTN_STAGES = W // 2 + 1 + NT


class _Spread:
    def __init__(self, gen, n_stages, n_slots, never):
        self.gen, self.n_stages, self.n_slots, self.never = gen, n_stages, n_slots, never
        self.slot = self.done = 0
        self.pending = []

    def step(self, part):
        if self.pending:
            tied = jnp.concatenate(self.pending, axis=0)
            n = tied.shape[0]
            head = jnp.where(self.never, tied, part[:n])
            part = head if n == part.shape[0] else jnp.concatenate([head, part[n:]], axis=0)
        self.pending = []
        self.slot += 1
        while self.done < min(self.n_stages, self.n_stages * self.slot // (self.n_slots - 1)):
            self.pending += next(self.gen)
            self.done += 1
        return part


def _pack(x):
    return pltpu.bitcast(x.astype(BF16), U32)


def _load_bf16(ref, rows, cols):
    if ref.dtype == BF16:
        return ref[rows, cols]
    return pltpu.bitcast(ref[rows.start // 2:rows.stop // 2, cols], BF16)


def _kernel(x_hbm, wqkv_hbm, wo_hbm, wg_hbm, wu_hbm, wd_hbm, c_ref, wmod_hbm, out_hbm,
            x_v, wqkv_raw, wq_v, wk_v, wv_v, wo_raw, wo_v, wg_v, wu_v, wd_v, wmod_v, sc_v, mod_v,
            q_v, k_v, v_v, o_v, act_v, ha_v, h_v, x1_v, accg_v, accu_v, out_v, zero_s, sems, out_sems):
    n_a = S // TA
    zero_s[0] = 0
    copies = {}

    def add_copy(name, src, dst):
        copies[name] = pltpu.make_async_copy(src, dst, sems.at[len(copies)])

    for p in range(3):
        add_copy(("w", p), wqkv_hbm.at[:, pl.ds(p * D, D)], wqkv_raw.at[p])
    for s in range(n_a):
        add_copy(("x", s), x_hbm.at[pl.ds(s * TA, TA)], x_v.at[pl.ds(s * TA, TA)])
    mod_chunks = [br * D + lo for lo in range(0, D, MA) for br in range(2)]
    for lo in mod_chunks:
        add_copy(("mod", lo), wmod_hbm.at[:, pl.ds(lo, MA)], wmod_v.at[:, pl.ds(lo, MA)])
    add_copy("mod_b", wmod_hbm.at[:, pl.ds(2 * D, 4 * D)], wmod_v.at[:, pl.ds(2 * D, 4 * D)])
    add_copy("wo", wo_hbm, wo_raw)
    add_copy("wg", wg_hbm, wg_v)
    add_copy("wu", wu_hbm, wu_v)
    add_copy("wd", wd_hbm, wd_v)

    def start(*names):
        for name in names:
            copies[name].start()

    def wait(*names):
        for name in names:
            copies[name].wait()

    def never(r0):
        return lax.broadcasted_iota(jnp.int32, (1, LANES), 1) + r0 < 0

    def silu_c():
        return _silu(c_ref[...].astype(F32)).astype(BF16)

    def mod_row(i):
        return mod_v[0:1, i * D:(i + 1) * D]

    def mod_b_stages():
        sc = silu_c().astype(F32)
        for lo in range(0, D, LANES):
            sc_v[lo:lo + LANES, :] = jnp.broadcast_to(sc[:, lo:lo + LANES], (LANES, LANES)).T
        for lo in range(2 * D, 6 * D, LANES):
            acc = None
            for r in range(0, D, MB):
                part = wmod_v[r:r + MB, lo:lo + LANES].astype(F32) * sc_v[r:r + MB, :]
                acc = part if acc is None else acc + part
            row = jnp.sum(acc, axis=0, keepdims=True).astype(BF16).astype(F32)
            row = jnp.broadcast_to(row, (8, LANES))
            mod_v[:, lo:lo + LANES] = row
            yield [row]

    def lane_tiles(v):
        return [v[:, j * LANES:(j + 1) * LANES] for j in range(v.shape[1] // LANES)]

    def ln_stages(src, dst, r0, n_rows, shift, scale):
        for r in range(r0, r0 + n_rows, LB):
            h = _layernorm(src[r:r + LB, :].astype(F32)) * (1.0 + mod_row(scale)) + mod_row(shift)
            h = _pack(h)
            dst[r // 2:(r + LB) // 2, :] = h
            yield [pltpu.bitcast(t, F32) for t in lane_tiles(h)]

    def permute_rows_of(p, r):
        lane = lax.broadcasted_iota(jnp.int32, (PR // 2, LANES), 1)
        t = [_pack(wqkv_raw[p, pl.ds(2 * r, PR), j * LANES:(j + 1) * LANES]) for j in range(NT)]
        for b in range(3):
            sh = 4 << b
            low = (lane & sh) == 0
            for j in range(NT):
                if j & (1 << b):
                    continue
                lo_t, hi_t = t[j], t[j | (1 << b)]
                t[j] = jnp.where(low, lo_t, pltpu.roll(hi_t, sh, 1))
                t[j | (1 << b)] = jnp.where(low, pltpu.roll(lo_t, LANES - sh, 1), hi_t)
        for j in range(NT):
            (wq_v, wk_v, wv_v)[p][pl.ds(r, PR // 2), j * LANES:(j + 1) * LANES] = t[j]
        return [pltpu.bitcast(tj, F32) for tj in t]

    def permute_stages(p):
        for r in range(0, D // 2, PR // 2):
            yield permute_rows_of(p, r)

    def wo_stages():
        for i in range(NT):
            done = []
            for hh in range(4):
                for jq in range(NT // 4):
                    pieces = []
                    for j in range(4 * jq, 4 * jq + 4):
                        src = (4 * j + hh) * DH + 4 * i
                        grp = wo_raw[src // 16 * 16:src // 16 * 16 + 16, :].astype(F32)
                        pieces.append(grp[src % 16:src % 16 + 4])
                    dst = i * LANES + hh * DH + jq * 16
                    blk = _pack(jnp.concatenate(pieces, axis=0))
                    wo_v[dst // 2:dst // 2 + 8, :] = blk
                    done += [pltpu.bitcast(t, F32) for t in lane_tiles(blk)]
            yield done

    def matmul_piece(lhs_ref, w_ref, lo, acc_ref, side):
        n_k = lhs_ref.shape[1] // KP
        for i in range(n_k):
            ks = slice(i * KP, (i + 1) * KP)
            part = jnp.dot(pltpu.bitcast(lhs_ref[:, ks], BF16), _load_bf16(w_ref, ks, slice(lo, lo + NP)),
                           preferred_element_type=F32)
            if i > 0:
                part = acc_ref[...] + part
            if side is not None:
                part = side.step(part)
            if i == n_k - 1:
                return part
            acc_ref[...] = part

    def project(p, s, side=None):
        dst, off = ((q_v, 0), (k_v, HALO), (v_v, HALO))[p]
        r0 = s * TA
        for n, lo in enumerate(range(0, D, NP)):
            acc = (accg_v, accu_v)[n % 2].at[0:TA]
            dst[r0 + off:r0 + off + TA, lo:lo + NP] = matmul_piece(
                ha_v.at[r0 // 2:(r0 + TA) // 2], (wq_v, wk_v, wv_v)[p], lo, acc, side)

    lane_a = lax.broadcasted_iota(jnp.int32, (RB, LANES), 1)
    row_a = lax.broadcasted_iota(jnp.int32, (RB, LANES), 0)
    even1 = (lane_a & 1) == 0
    even2 = (lane_a & 2) == 0
    scale = DH ** -0.5

    def shifted(ref, r0, i, c):
        win = ref[pl.ds(r0, RB + HALO), i * LANES:(i + 1) * LANES]
        lo = HALO - 8 - DIL * c
        blk = win[lo:lo + RB + 8]
        return blk[8:], blk[:RB]

    def attn_block(r0, half):
        logit = [None] * W
        pos = row_a + r0
        for c in range(W // 2):
            ws = (c, c + W // 2)
            for i in range(NT):
                qi = q_v[pl.ds(r0, RB), i * LANES:(i + 1) * LANES]
                for w, kw in zip(ws, shifted(k_v, r0, i, c)):
                    logit[w] = qi * kw if i == 0 else logit[w] + qi * kw
            for w in ws:
                s = logit[w]
                s = s + jnp.where(even1, pltpu.roll(s, LANES - 1, 1), pltpu.roll(s, 1, 1))
                s = s + jnp.where(even2, pltpu.roll(s, LANES - 2, 1), pltpu.roll(s, 2, 1))
                s = s * scale
                logit[w] = s if w == 0 else jnp.where(pos >= DIL * w, s, -1e9)
            yield [logit[w] for w in ws]
        m = logit[0]
        for w in range(1, W):
            m = jnp.maximum(m, logit[w])
        e = [jnp.exp(s - m) for s in logit]
        den = e[0]
        for w in range(1, W):
            den = den + e[w]
        inv = 1.0 / den
        prob = [ew * inv for ew in e]
        yield [inv]
        for i in range(NT):
            acc = None
            for c in range(W // 2):
                for w, vw in zip((c, c + W // 2), shifted(v_v, r0, i, c)):
                    acc = prob[w] * vw if acc is None else acc + prob[w] * vw
            o_v[pl.ds(half, RB // 2), i * LANES:(i + 1) * LANES] = _pack(acc)
            yield [acc]

    def attn_rows(r0, n_blocks):
        for b in range(n_blocks):
            start_row = r0 + b * RB
            if isinstance(r0, int):
                yield from attn_block(start_row, start_row // 2)
            else:
                yield from attn_block(pl.multiple_of(start_row, RB), pl.multiple_of(start_row // 2, RB // 2))

    start(("w", 0), ("x", 0))
    wait(("w", 0))
    start(*[("mod", lo) for lo in mod_chunks])

    def permute_q(r, carry):
        permute_rows_of(0, pl.multiple_of(r * PR, PR // 2))
        permute_rows_of(0, pl.multiple_of(r * PR + PR // 2, PR // 2))
        return carry
    lax.fori_loop(0, D // PR // 2, permute_q, 0)
    wait(("x", 0))
    x1_v[0:TA, :] = _layernorm(x_v[0:TA, :].astype(F32))
    sc_rows = jnp.broadcast_to(silu_c(), (MOD_ROWS, D))
    late = [("x", s) for s in range(1, n_a)] + [("w", 1)]
    for i, lo in enumerate(mod_chunks):
        wait(("mod", lo))
        if i % 2 == 1 and late:
            start(late.pop(0))
        r = jnp.dot(sc_rows, wmod_v[:, lo:lo + MA], preferred_element_type=F32)
        mod_v[:, lo:lo + MA] = r[0:8].astype(BF16).astype(F32)
        if i % 2 == 1:
            cols = slice(lo - D, lo - D + MA)
            ha_v[0:TA // 2, cols] = _pack(x1_v[0:TA, cols] * (1.0 + mod_row(1)[:, cols]) + mod_row(0)[:, cols])
    start(*late)

    slots = D // NP * (D // KP)
    zero = zero_s[0]
    for s in range(n_a - 1):
        wait(("x", s + 1))
        if s == 1:
            start(("w", 2))
        project(0, s, _Spread(ln_stages(x_v, ha_v, (s + 1) * TA, TA, 0, 1), TA // LB, slots, never(zero)))
    wait(("w", 1))
    start("mod_b", "wo")
    project(0, n_a - 1, _Spread(permute_stages(1), D // PR, slots, never(zero)))
    wait(("w", 2))
    start("wg", "wu", "wd")
    project(1, 0, _Spread(permute_stages(2), D // PR, slots, never(zero)))
    wait("mod_b", "wo")
    project(1, 1, _Spread(wo_stages(), NT, slots, never(zero)))
    side = _Spread(mod_b_stages(), 4 * D // LANES, (n_a - 2) * slots, never(zero))
    for s in range(2, n_a):
        project(1, s, side)
    first = TC // TA
    for s in range(first):
        project(2, s)
    k_v[0:HALO, :] = jnp.broadcast_to(k_v[HALO:HALO + 1, :], (HALO, D))
    v_v[0:HALO, :] = jnp.broadcast_to(v_v[HALO:HALO + 1, :], (HALO, D))
    side = _Spread(attn_rows(0, TC // RB), TC // RB * ATTN_STAGES, (n_a - first) * slots, never(zero))
    for s in range(first, n_a):
        project(2, s, side)
    wait("wg", "wu", "wd")

    def out_copy(t, slot):
        return pltpu.make_async_copy(out_v.at[slot], out_hbm.at[pl.ds(t * TC, TC)], out_sems.at[slot])

    n_c = S // TC

    def phase_c(t, carry):
        rows = pl.ds(pl.multiple_of(t * TC, TC), TC)
        slot = t % 2

        @pl.when(t >= 2)
        def _():
            out_copy(t - 2, slot).wait()
        for n, lo in enumerate(range(0, D, NP)):
            a = matmul_piece(o_v.at[pl.ds(pl.multiple_of(t * (TC // 2), TC // 2), TC // 2)], wo_v, lo, (accg_v, accu_v)[n % 2], None)
            x1_v[0:TC, lo:lo + NP] = x_v[rows, lo:lo + NP].astype(F32) + mod_row(2)[:, lo:lo + NP] * a
        h_v[...] = _pack(_layernorm(x1_v[0:TC, :]) * (1.0 + mod_row(4)) + mod_row(3))
        nxt = jnp.minimum(t + 1, n_c - 1) * TC
        n_slots = 3 * (F // NP) * (D // KP)
        side = _Spread(attn_rows(nxt, TC // RB), TC // RB * ATTN_STAGES, n_slots, never(nxt))
        for lo in range(0, F, NP):
            accg_v[...] = matmul_piece(h_v, wg_v, lo, accg_v, side)
            u = matmul_piece(h_v, wu_v, lo, accu_v, side)
            act_v[:, lo:lo + NP] = _pack(_silu(accg_v[...]) * u)
        for n, lo in enumerate(range(0, D, NP)):
            y = matmul_piece(act_v, wd_v, lo, (accg_v, accu_v)[n % 2], side)
            out_v[slot, :, lo:lo + NP] = (x1_v[0:TC, lo:lo + NP] + mod_row(5)[:, lo:lo + NP] * y).astype(BF16)
        out_copy(t, slot).start()
        return carry
    lax.fori_loop(0, n_c, phase_c, 0)
    for t in range(n_c - 2, n_c):
        out_copy(t, t % 2).wait()


@jax.jit
def pallas_adaLN_cond__sliding_local_dilated__swiglu_ffn__prompt_kernel(
    A_x: jax.Array,
    A_wqkv: jax.Array,
    A_wo: jax.Array,
    B_x: jax.Array,
    B_w_gate: jax.Array,
    B_w_up: jax.Array,
    B_w_down: jax.Array,
    c: jax.Array,
    w_mod: jax.Array,
):
    del B_x
    hbm = pl.BlockSpec(memory_space=pl.ANY)
    out = pl.pallas_call(
        _kernel,
        out_shape=jax.ShapeDtypeStruct((S, D), BF16),
        in_specs=[hbm, hbm, hbm, hbm, hbm, hbm, pl.BlockSpec(memory_space=pltpu.VMEM), hbm],
        out_specs=hbm,
        scratch_shapes=[
            pltpu.VMEM((S, D), BF16),
            pltpu.VMEM((3, D, D), BF16),
            pltpu.VMEM((D // 2, D), U32),
            pltpu.VMEM((D // 2, D), U32),
            pltpu.VMEM((D // 2, D), U32),
            pltpu.VMEM((D, D), BF16),
            pltpu.VMEM((D // 2, D), U32),
            pltpu.VMEM((D, F), BF16),
            pltpu.VMEM((D, F), BF16),
            pltpu.VMEM((F, D), BF16),
            pltpu.VMEM((D, 6 * D), BF16),
            pltpu.VMEM((D, LANES), F32),
            pltpu.VMEM((8, 6 * D), F32),
            pltpu.VMEM((S, D), F32),
            pltpu.VMEM((S + HALO, D), F32),
            pltpu.VMEM((S + HALO, D), F32),
            pltpu.VMEM((S // 2, D), U32),
            pltpu.VMEM((TC // 2, F), U32),
            pltpu.VMEM((S // 2, D), U32),
            pltpu.VMEM((TC // 2, D), U32),
            pltpu.VMEM((max(TA, TC), D), F32),
            pltpu.VMEM((max(TA, TC), NP), F32),
            pltpu.VMEM((max(TA, TC), NP), F32),
            pltpu.VMEM((2, TC, D), BF16),
            pltpu.SMEM((1,), jnp.int32),
            pltpu.SemaphoreType.DMA((8 + S // TA + 2 * D // MA,)),
            pltpu.SemaphoreType.DMA((2,)),
        ],
        compiler_params=pltpu.CompilerParams(vmem_limit_bytes=120 * 1024 * 1024),
    )(A_x.reshape(S, D), A_wqkv, A_wo, B_w_gate, B_w_up, B_w_down, c, w_mod)
    return out.reshape(1, S, D)
```

```python
import jax
import jax.numpy as jnp
from jax import lax
from jax.experimental import pallas as pl
from jax.experimental.pallas import tpu as pltpu

S, D, F = 2048, 1024, 3584
H, DH, W, DIL = 32, 32, 8, 2
LANES = 128
NT = D // LANES
HALO = 16
TA = 512
RB = 32
TC = 512
NP, KP = 128, 512
PR = 64
LB = 32
MOD_ROWS, MA, MB = 16, 256, 32
EPS = 1e-5
F32, BF16, U32 = jnp.float32, jnp.bfloat16, jnp.uint32


def _layernorm(x):
    m = jnp.mean(x, axis=-1, keepdims=True)
    xc = x - m
    v = jnp.mean(xc * xc, axis=-1, keepdims=True)
    return xc * lax.rsqrt(v + EPS)


def _silu(x):
    return x * (1.0 / (1.0 + jnp.exp(-x)))


ATTN_STAGES = W // 2 + 1 + NT


class _Spread:
    def __init__(self, gen, n_stages, n_slots, never):
        self.gen, self.n_stages, self.n_slots, self.never = gen, n_stages, n_slots, never
        self.slot = self.done = 0
        self.pending = []

    def step(self, part):
        if self.pending:
            tied = jnp.concatenate(self.pending, axis=0)
            n = tied.shape[0]
            head = jnp.where(self.never, tied, part[:n])
            part = head if n == part.shape[0] else jnp.concatenate([head, part[n:]], axis=0)
        self.pending = []
        self.slot += 1
        while self.done < min(self.n_stages, self.n_stages * self.slot // (self.n_slots - 1)):
            self.pending += next(self.gen)
            self.done += 1
        return part


def _pack(x):
    return pltpu.bitcast(x.astype(BF16), U32)


def _load_bf16(ref, rows, cols):
    if ref.dtype == BF16:
        return ref[rows, cols]
    return pltpu.bitcast(ref[rows.start // 2:rows.stop // 2, cols], BF16)


def _kernel(x_hbm, wqkv_hbm, wo_hbm, wg_hbm, wu_hbm, wd_hbm, c_ref, wmod_hbm, out_hbm,
            x_v, wqkv_raw, wq_v, wk_v, wv_v, wo_raw, wo_v, wg_v, wu_v, wd_v, wmod_v, sc_v, mod_v,
            q_v, k_v, v_v, o_v, act_v, ha_v, h_v, x1_v, accg_v, accu_v, out_v, zero_s, sems, out_sems):
    n_a = S // TA
    zero_s[0] = 0
    copies = {}

    def add_copy(name, src, dst):
        copies[name] = pltpu.make_async_copy(src, dst, sems.at[len(copies)])

    for p in range(3):
        add_copy(("w", p), wqkv_hbm.at[:, pl.ds(p * D, D)], wqkv_raw.at[p])
    for s in range(n_a):
        add_copy(("x", s), x_hbm.at[pl.ds(s * TA, TA)], x_v.at[pl.ds(s * TA, TA)])
    mod_chunks = [br * D + lo for lo in range(0, D, MA) for br in range(2)]
    for lo in mod_chunks:
        add_copy(("mod", lo), wmod_hbm.at[:, pl.ds(lo, MA)], wmod_v.at[:, pl.ds(lo, MA)])
    add_copy("mod_b", wmod_hbm.at[:, pl.ds(2 * D, 4 * D)], wmod_v.at[:, pl.ds(2 * D, 4 * D)])
    add_copy("wo", wo_hbm, wo_raw)
    add_copy("wg", wg_hbm, wg_v)
    add_copy("wu", wu_hbm, wu_v)
    add_copy("wd", wd_hbm, wd_v)

    def start(*names):
        for name in names:
            copies[name].start()

    def wait(*names):
        for name in names:
            copies[name].wait()

    def never(r0):
        return lax.broadcasted_iota(jnp.int32, (1, LANES), 1) + r0 < 0

    def silu_c():
        return _silu(c_ref[...].astype(F32)).astype(BF16)

    def mod_row(i):
        return mod_v[0:1, i * D:(i + 1) * D]

    def mod_b_stages():
        sc = silu_c().astype(F32)
        for lo in range(0, D, LANES):
            sc_v[lo:lo + LANES, :] = jnp.broadcast_to(sc[:, lo:lo + LANES], (LANES, LANES)).T
        for lo in range(2 * D, 6 * D, LANES):
            acc = None
            for r in range(0, D, MB):
                part = wmod_v[r:r + MB, lo:lo + LANES].astype(F32) * sc_v[r:r + MB, :]
                acc = part if acc is None else acc + part
            row = jnp.sum(acc, axis=0, keepdims=True).astype(BF16).astype(F32)
            row = jnp.broadcast_to(row, (8, LANES))
            mod_v[:, lo:lo + LANES] = row
            yield [row]

    def lane_tiles(v):
        return [v[:, j * LANES:(j + 1) * LANES] for j in range(v.shape[1] // LANES)]

    def ln_stages(src, dst, r0, n_rows, shift, scale):
        for r in range(r0, r0 + n_rows, LB):
            h = _layernorm(src[r:r + LB, :].astype(F32)) * (1.0 + mod_row(scale)) + mod_row(shift)
            h = _pack(h)
            dst[r // 2:(r + LB) // 2, :] = h
            yield [pltpu.bitcast(t, F32) for t in lane_tiles(h)]

    def permute_rows_of(p, r):
        lane = lax.broadcasted_iota(jnp.int32, (PR // 2, LANES), 1)
        t = [_pack(wqkv_raw[p, pl.ds(2 * r, PR), j * LANES:(j + 1) * LANES]) for j in range(NT)]
        for b in range(3):
            sh = 4 << b
            low = (lane & sh) == 0
            for j in range(NT):
                if j & (1 << b):
                    continue
                lo_t, hi_t = t[j], t[j | (1 << b)]
                t[j] = jnp.where(low, lo_t, pltpu.roll(hi_t, sh, 1))
                t[j | (1 << b)] = jnp.where(low, pltpu.roll(lo_t, LANES - sh, 1), hi_t)
        for j in range(NT):
            (wq_v, wk_v, wv_v)[p][pl.ds(r, PR // 2), j * LANES:(j + 1) * LANES] = t[j]
        return [pltpu.bitcast(tj, F32) for tj in t]

    def permute_stages(p):
        for r in range(0, D // 2, PR // 2):
            yield permute_rows_of(p, r)

    def wo_stages():
        for i in range(NT):
            done = []
            for hh in range(4):
                for jq in range(NT // 4):
                    pieces = []
                    for j in range(4 * jq, 4 * jq + 4):
                        src = (4 * j + hh) * DH + 4 * i
                        grp = wo_raw[src // 16 * 16:src // 16 * 16 + 16, :].astype(F32)
                        pieces.append(grp[src % 16:src % 16 + 4])
                    dst = i * LANES + hh * DH + jq * 16
                    blk = _pack(jnp.concatenate(pieces, axis=0))
                    wo_v[dst // 2:dst // 2 + 8, :] = blk
                    done += [pltpu.bitcast(t, F32) for t in lane_tiles(blk)]
            yield done

    def matmul_piece(lhs_ref, w_ref, lo, acc_ref, side):
        n_k = lhs_ref.shape[1] // KP
        for i in range(n_k):
            ks = slice(i * KP, (i + 1) * KP)
            part = jnp.dot(pltpu.bitcast(lhs_ref[:, ks], BF16), _load_bf16(w_ref, ks, slice(lo, lo + NP)),
                           preferred_element_type=F32)
            if i > 0:
                part = acc_ref[...] + part
            if side is not None:
                part = side.step(part)
            if i == n_k - 1:
                return part
            acc_ref[...] = part

    def project(p, s, side=None):
        dst, off = ((q_v, 0), (k_v, HALO), (v_v, HALO))[p]
        r0 = s * TA
        for n, lo in enumerate(range(0, D, NP)):
            acc = (accg_v, accu_v)[n % 2].at[0:TA]
            dst[r0 + off:r0 + off + TA, lo:lo + NP] = matmul_piece(
                ha_v.at[r0 // 2:(r0 + TA) // 2], (wq_v, wk_v, wv_v)[p], lo, acc, side)

    lane_a = lax.broadcasted_iota(jnp.int32, (RB, LANES), 1)
    row_a = lax.broadcasted_iota(jnp.int32, (RB, LANES), 0)
    even1 = (lane_a & 1) == 0
    even2 = (lane_a & 2) == 0
    scale = DH ** -0.5

    def shifted(ref, r0, i, c):
        win = ref[pl.ds(r0, RB + HALO), i * LANES:(i + 1) * LANES]
        lo = HALO - 8 - DIL * c
        blk = win[lo:lo + RB + 8]
        return blk[8:], blk[:RB]

    def attn_block(r0, half):
        logit = [None] * W
        pos = row_a + r0
        for c in range(W // 2):
            ws = (c, c + W // 2)
            for i in range(NT):
                qi = q_v[pl.ds(r0, RB), i * LANES:(i + 1) * LANES]
                for w, kw in zip(ws, shifted(k_v, r0, i, c)):
                    logit[w] = qi * kw if i == 0 else logit[w] + qi * kw
            for w in ws:
                s = logit[w]
                s = s + jnp.where(even1, pltpu.roll(s, LANES - 1, 1), pltpu.roll(s, 1, 1))
                s = s + jnp.where(even2, pltpu.roll(s, LANES - 2, 1), pltpu.roll(s, 2, 1))
                s = s * scale
                logit[w] = s if w == 0 else jnp.where(pos >= DIL * w, s, -1e9)
            yield [logit[w] for w in ws]
        m = logit[0]
        for w in range(1, W):
            m = jnp.maximum(m, logit[w])
        e = [jnp.exp(s - m) for s in logit]
        den = e[0]
        for w in range(1, W):
            den = den + e[w]
        inv = 1.0 / den
        prob = [ew * inv for ew in e]
        yield [inv]
        for i in range(NT):
            acc = None
            for c in range(W // 2):
                for w, vw in zip((c, c + W // 2), shifted(v_v, r0, i, c)):
                    acc = prob[w] * vw if acc is None else acc + prob[w] * vw
            o_v[pl.ds(half, RB // 2), i * LANES:(i + 1) * LANES] = _pack(acc)
            yield [acc]

    def attn_rows(r0, n_blocks):
        for b in range(n_blocks):
            start_row = r0 + b * RB
            if isinstance(r0, int):
                yield from attn_block(start_row, start_row // 2)
            else:
                yield from attn_block(pl.multiple_of(start_row, RB), pl.multiple_of(start_row // 2, RB // 2))

    start(("w", 0), ("x", 0))
    wait(("w", 0))
    start(*[("mod", lo) for lo in mod_chunks])

    def permute_q(r, carry):
        permute_rows_of(0, pl.multiple_of(r * PR, PR // 2))
        permute_rows_of(0, pl.multiple_of(r * PR + PR // 2, PR // 2))
        return carry
    lax.fori_loop(0, D // PR // 2, permute_q, 0)
    wait(("x", 0))
    x1_v[0:TA, :] = _layernorm(x_v[0:TA, :].astype(F32))
    sc_rows = jnp.broadcast_to(silu_c(), (MOD_ROWS, D))
    for i, lo in enumerate(mod_chunks):
        wait(("mod", lo))
        if i == len(mod_chunks) - 1:
            start(("x", 1), ("x", 2))
        r = jnp.dot(sc_rows, wmod_v[:, lo:lo + MA], preferred_element_type=F32)
        mod_v[:, lo:lo + MA] = r[0:8].astype(BF16).astype(F32)
        if i % 2 == 1:
            cols = slice(lo - D, lo - D + MA)
            ha_v[0:TA // 2, cols] = _pack(x1_v[0:TA, cols] * (1.0 + mod_row(1)[:, cols]) + mod_row(0)[:, cols])

    slots = D // NP * (D // KP)
    zero = zero_s[0]

    def next_ln(s):
        for _ in range(TA // LB):
            yield []
        wait(("x", s))
        if s == 1:
            start(*[("x", i) for i in range(3, n_a)], ("w", 1), ("w", 2))
        if s == n_a - 1:
            start("wo", "mod_b")
        yield from ln_stages(x_v, ha_v, s * TA, TA, 0, 1)

    for s in range(n_a - 1):
        project(0, s, _Spread(next_ln(s + 1), 2 * (TA // LB), slots, never(zero)))
    wait(("w", 1))
    project(0, n_a - 1, _Spread(permute_stages(1), D // PR, slots, never(zero)))
    wait(("w", 2))
    project(1, 0, _Spread(permute_stages(2), D // PR, slots, never(zero)))
    wait("wo")
    project(1, 1, _Spread(wo_stages(), NT, slots, never(zero)))
    wait("mod_b")
    start("wg", "wu", "wd")
    side = _Spread(mod_b_stages(), 4 * D // LANES, (n_a - 2) * slots, never(zero))
    for s in range(2, n_a):
        project(1, s, side)
    first = TC // TA
    for s in range(first):
        project(2, s)
    k_v[0:HALO, :] = jnp.broadcast_to(k_v[HALO:HALO + 1, :], (HALO, D))
    v_v[0:HALO, :] = jnp.broadcast_to(v_v[HALO:HALO + 1, :], (HALO, D))
    side = _Spread(attn_rows(0, TC // RB), TC // RB * ATTN_STAGES, (n_a - first) * slots, never(zero))
    for s in range(first, n_a):
        project(2, s, side)
    wait("wg", "wu", "wd")

    def out_copy(t, slot, half):
        cols = pl.ds(half * (D // 2), D // 2)
        return pltpu.make_async_copy(out_v.at[slot, :, cols], out_hbm.at[pl.ds(t * TC, TC), cols],
                                     out_sems.at[slot, half])

    n_c = S // TC

    def phase_c(t, carry):
        rows = pl.ds(pl.multiple_of(t * TC, TC), TC)
        slot = t % 2

        @pl.when(t >= 2)
        def _():
            out_copy(t - 2, slot, 0).wait()
            out_copy(t - 2, slot, 1).wait()
        for n, lo in enumerate(range(0, D, NP)):
            a = matmul_piece(o_v.at[pl.ds(pl.multiple_of(t * (TC // 2), TC // 2), TC // 2)], wo_v, lo, (accg_v, accu_v)[n % 2], None)
            x1_v[0:TC, lo:lo + NP] = x_v[rows, lo:lo + NP].astype(F32) + mod_row(2)[:, lo:lo + NP] * a
        h_v[...] = _pack(_layernorm(x1_v[0:TC, :]) * (1.0 + mod_row(4)) + mod_row(3))
        nxt = jnp.minimum(t + 1, n_c - 1) * TC
        n_slots = 3 * (F // NP) * (D // KP)
        side = _Spread(attn_rows(nxt, TC // RB), TC // RB * ATTN_STAGES, n_slots, never(nxt))
        for lo in range(0, F, NP):
            accg_v[...] = matmul_piece(h_v, wg_v, lo, accg_v, side)
            u = matmul_piece(h_v, wu_v, lo, accu_v, side)
            act_v[:, lo:lo + NP] = _pack(_silu(accg_v[...]) * u)
        for n, lo in enumerate(range(0, D, NP)):
            y = matmul_piece(act_v, wd_v, lo, (accg_v, accu_v)[n % 2], side)
            out_v[slot, :, lo:lo + NP] = (x1_v[0:TC, lo:lo + NP] + mod_row(5)[:, lo:lo + NP] * y).astype(BF16)
            if (lo + NP) % (D // 2) == 0:
                out_copy(t, slot, lo // (D // 2)).start()
        return carry
    lax.fori_loop(0, n_c, phase_c, 0)
    for t in range(n_c - 2, n_c):
        out_copy(t, t % 2, 0).wait()
        out_copy(t, t % 2, 1).wait()


@jax.jit
def pallas_adaLN_cond__sliding_local_dilated__swiglu_ffn__prompt_kernel(
    A_x: jax.Array,
    A_wqkv: jax.Array,
    A_wo: jax.Array,
    B_x: jax.Array,
    B_w_gate: jax.Array,
    B_w_up: jax.Array,
    B_w_down: jax.Array,
    c: jax.Array,
    w_mod: jax.Array,
):
    del B_x
    hbm = pl.BlockSpec(memory_space=pl.ANY)
    out = pl.pallas_call(
        _kernel,
        out_shape=jax.ShapeDtypeStruct((S, D), BF16),
        in_specs=[hbm, hbm, hbm, hbm, hbm, hbm, pl.BlockSpec(memory_space=pltpu.VMEM), hbm],
        out_specs=hbm,
        scratch_shapes=[
            pltpu.VMEM((S, D), BF16),
            pltpu.VMEM((3, D, D), BF16),
            pltpu.VMEM((D // 2, D), U32),
            pltpu.VMEM((D // 2, D), U32),
            pltpu.VMEM((D // 2, D), U32),
            pltpu.VMEM((D, D), BF16),
            pltpu.VMEM((D // 2, D), U32),
            pltpu.VMEM((D, F), BF16),
            pltpu.VMEM((D, F), BF16),
            pltpu.VMEM((F, D), BF16),
            pltpu.VMEM((D, 6 * D), BF16),
            pltpu.VMEM((D, LANES), F32),
            pltpu.VMEM((8, 6 * D), F32),
            pltpu.VMEM((S, D), F32),
            pltpu.VMEM((S + HALO, D), F32),
            pltpu.VMEM((S + HALO, D), F32),
            pltpu.VMEM((S // 2, D), U32),
            pltpu.VMEM((TC // 2, F), U32),
            pltpu.VMEM((S // 2, D), U32),
            pltpu.VMEM((TC // 2, D), U32),
            pltpu.VMEM((max(TA, TC), D), F32),
            pltpu.VMEM((max(TA, TC), NP), F32),
            pltpu.VMEM((max(TA, TC), NP), F32),
            pltpu.VMEM((2, TC, D), BF16),
            pltpu.SMEM((1,), jnp.int32),
            pltpu.SemaphoreType.DMA((8 + S // TA + 2 * D // MA,)),
            pltpu.SemaphoreType.DMA((2, 2)),
        ],
        compiler_params=pltpu.CompilerParams(vmem_limit_bytes=120 * 1024 * 1024),
    )(A_x.reshape(S, D), A_wqkv, A_wo, B_w_gate, B_w_up, B_w_down, c, w_mod)
    return out.reshape(1, S, D)
```

```python
import jax
import jax.numpy as jnp
from jax import lax
from jax.experimental import pallas as pl
from jax.experimental.pallas import tpu as pltpu

S, D, F = 2048, 1024, 3584
H, DH, W, DIL = 32, 32, 8, 2
LANES = 128
NT = D // LANES
HALO = 16
TA = 512
RB = 32
TC = 512
NP, KP = 128, 512
PR = 64
LB = 32
MOD_ROWS, MA, MB = 16, 256, 32
OC = 256
EPS = 1e-5
F32, BF16, U32 = jnp.float32, jnp.bfloat16, jnp.uint32


def _layernorm(x):
    m = jnp.mean(x, axis=-1, keepdims=True)
    xc = x - m
    v = jnp.mean(xc * xc, axis=-1, keepdims=True)
    return xc * lax.rsqrt(v + EPS)


def _silu(x):
    return x * (1.0 / (1.0 + jnp.exp(-x)))


ATTN_STAGES = W // 2 + 1 + NT


class _Spread:
    def __init__(self, gen, n_stages, n_slots, never):
        self.gen, self.n_stages, self.n_slots, self.never = gen, n_stages, n_slots, never
        self.slot = self.done = 0
        self.pending = []

    def step(self, part):
        if self.pending:
            tied = jnp.concatenate(self.pending, axis=0)
            n = tied.shape[0]
            head = jnp.where(self.never, tied, part[:n])
            part = head if n == part.shape[0] else jnp.concatenate([head, part[n:]], axis=0)
        self.pending = []
        self.slot += 1
        while self.done < min(self.n_stages, self.n_stages * self.slot // (self.n_slots - 1)):
            self.pending += next(self.gen)
            self.done += 1
        return part


def _pack(x):
    return pltpu.bitcast(x.astype(BF16), U32)


def _load_bf16(ref, rows, cols):
    if ref.dtype == BF16:
        return ref[rows, cols]
    return pltpu.bitcast(ref[rows.start // 2:rows.stop // 2, cols], BF16)


def _kernel(x_hbm, wqkv_hbm, wo_hbm, wg_hbm, wu_hbm, wd_hbm, c_ref, wmod_hbm, out_hbm,
            x_v, wqkv_raw, wq_v, wk_v, wv_v, wo_raw, wo_v, wg_v, wu_v, wd_v, wmod_v, sc_v, mod_v,
            q_v, k_v, v_v, o_v, act_v, ha_v, h_v, x1_v, accg_v, accu_v, out_v, zero_s, sems, out_sems):
    n_a = S // TA
    zero_s[0] = 0
    copies = {}

    def add_copy(name, src, dst):
        copies[name] = pltpu.make_async_copy(src, dst, sems.at[len(copies)])

    for r in range(0, D, MA):
        add_copy(("wq", r), wqkv_hbm.at[pl.ds(r, MA), pl.ds(0, D)], wqkv_raw.at[0, pl.ds(r, MA)])
    for p in (1, 2):
        add_copy(("w", p), wqkv_hbm.at[:, pl.ds(p * D, D)], wqkv_raw.at[p])
    for s in range(n_a):
        add_copy(("x", s), x_hbm.at[pl.ds(s * TA, TA)], x_v.at[pl.ds(s * TA, TA)])
    for lo in range(0, 2 * D, MA):
        add_copy(("mod", lo), wmod_hbm.at[:, pl.ds(lo, MA)], wmod_v.at[:, pl.ds(lo, MA)])
    add_copy("mod_b", wmod_hbm.at[:, pl.ds(2 * D, 4 * D)], wmod_v.at[:, pl.ds(2 * D, 4 * D)])
    add_copy("wo", wo_hbm, wo_raw)
    add_copy("wg", wg_hbm, wg_v)
    add_copy("wu", wu_hbm, wu_v)
    add_copy("wd", wd_hbm, wd_v)

    def start(*names):
        for name in names:
            copies[name].start()

    def wait(*names):
        for name in names:
            copies[name].wait()

    def never(r0):
        return lax.broadcasted_iota(jnp.int32, (1, LANES), 1) + r0 < 0

    def silu_c():
        return _silu(c_ref[...].astype(F32)).astype(BF16)

    def mod_row(i):
        return mod_v[0:1, i * D:(i + 1) * D]

    def mod_b_stages():
        sc = silu_c().astype(F32)
        for lo in range(0, D, LANES):
            sc_v[lo:lo + LANES, :] = jnp.broadcast_to(sc[:, lo:lo + LANES], (LANES, LANES)).T
        for lo in range(2 * D, 6 * D, LANES):
            acc = None
            for r in range(0, D, MB):
                part = wmod_v[r:r + MB, lo:lo + LANES].astype(F32) * sc_v[r:r + MB, :]
                acc = part if acc is None else acc + part
            row = jnp.sum(acc, axis=0, keepdims=True).astype(BF16).astype(F32)
            row = jnp.broadcast_to(row, (8, LANES))
            mod_v[:, lo:lo + LANES] = row
            yield [row]

    def lane_tiles(v):
        return [v[:, j * LANES:(j + 1) * LANES] for j in range(v.shape[1] // LANES)]

    def ln_stages(src, dst, r0, n_rows, shift, scale):
        for r in range(r0, r0 + n_rows, LB):
            h = _layernorm(src[r:r + LB, :].astype(F32)) * (1.0 + mod_row(scale)) + mod_row(shift)
            h = _pack(h)
            dst[r // 2:(r + LB) // 2, :] = h
            yield [pltpu.bitcast(t, F32) for t in lane_tiles(h)]

    def permute_rows_of(p, r):
        lane = lax.broadcasted_iota(jnp.int32, (PR // 2, LANES), 1)
        t = [_pack(wqkv_raw[p, pl.ds(2 * r, PR), j * LANES:(j + 1) * LANES]) for j in range(NT)]
        for b in range(3):
            sh = 4 << b
            low = (lane & sh) == 0
            for j in range(NT):
                if j & (1 << b):
                    continue
                lo_t, hi_t = t[j], t[j | (1 << b)]
                t[j] = jnp.where(low, lo_t, pltpu.roll(hi_t, sh, 1))
                t[j | (1 << b)] = jnp.where(low, pltpu.roll(lo_t, LANES - sh, 1), hi_t)
        for j in range(NT):
            (wq_v, wk_v, wv_v)[p][pl.ds(r, PR // 2), j * LANES:(j + 1) * LANES] = t[j]
        return [pltpu.bitcast(tj, F32) for tj in t]

    def permute_stages(p, lo=0, hi=D):
        for r in range(lo // 2, hi // 2, PR // 2):
            yield permute_rows_of(p, r)

    def wo_stages():
        for i in range(NT):
            done = []
            for hh in range(4):
                for jq in range(NT // 4):
                    pieces = []
                    for j in range(4 * jq, 4 * jq + 4):
                        src = (4 * j + hh) * DH + 4 * i
                        grp = wo_raw[src // 16 * 16:src // 16 * 16 + 16, :].astype(F32)
                        pieces.append(grp[src % 16:src % 16 + 4])
                    dst = i * LANES + hh * DH + jq * 16
                    blk = _pack(jnp.concatenate(pieces, axis=0))
                    wo_v[dst // 2:dst // 2 + 8, :] = blk
                    done += [pltpu.bitcast(t, F32) for t in lane_tiles(blk)]
            yield done

    def matmul_piece(lhs_ref, w_ref, lo, acc_ref, side):
        n_k = lhs_ref.shape[1] // KP
        for i in range(n_k):
            ks = slice(i * KP, (i + 1) * KP)
            part = jnp.dot(pltpu.bitcast(lhs_ref[:, ks], BF16), _load_bf16(w_ref, ks, slice(lo, lo + NP)),
                           preferred_element_type=F32)
            if i > 0:
                part = acc_ref[...] + part
            if side is not None:
                part = side.step(part)
            if i == n_k - 1:
                return part
            acc_ref[...] = part

    def project(p, s, side=None):
        dst, off = ((q_v, 0), (k_v, HALO), (v_v, HALO))[p]
        r0 = s * TA
        for n, lo in enumerate(range(0, D, NP)):
            acc = (accg_v, accu_v)[n % 2].at[0:TA]
            dst[r0 + off:r0 + off + TA, lo:lo + NP] = matmul_piece(
                ha_v.at[r0 // 2:(r0 + TA) // 2], (wq_v, wk_v, wv_v)[p], lo, acc, side)

    lane_a = lax.broadcasted_iota(jnp.int32, (RB, LANES), 1)
    row_a = lax.broadcasted_iota(jnp.int32, (RB, LANES), 0)
    even1 = (lane_a & 1) == 0
    even2 = (lane_a & 2) == 0
    scale = DH ** -0.5

    def shifted(ref, r0, i, c):
        win = ref[pl.ds(r0, RB + HALO), i * LANES:(i + 1) * LANES]
        lo = HALO - 8 - DIL * c
        blk = win[lo:lo + RB + 8]
        return blk[8:], blk[:RB]

    def attn_block(r0, half):
        logit = [None] * W
        pos = row_a + r0
        for c in range(W // 2):
            ws = (c, c + W // 2)
            for i in range(NT):
                qi = q_v[pl.ds(r0, RB), i * LANES:(i + 1) * LANES]
                for w, kw in zip(ws, shifted(k_v, r0, i, c)):
                    logit[w] = qi * kw if i == 0 else logit[w] + qi * kw
            for w in ws:
                s = logit[w]
                s = s + jnp.where(even1, pltpu.roll(s, LANES - 1, 1), pltpu.roll(s, 1, 1))
                s = s + jnp.where(even2, pltpu.roll(s, LANES - 2, 1), pltpu.roll(s, 2, 1))
                s = s * scale
                logit[w] = s if w == 0 else jnp.where(pos >= DIL * w, s, -1e9)
            yield [logit[w] for w in ws]
        m = logit[0]
        for w in range(1, W):
            m = jnp.maximum(m, logit[w])
        e = [jnp.exp(s - m) for s in logit]
        den = e[0]
        for w in range(1, W):
            den = den + e[w]
        inv = 1.0 / den
        prob = [ew * inv for ew in e]
        yield [inv]
        for i in range(NT):
            acc = None
            for c in range(W // 2):
                for w, vw in zip((c, c + W // 2), shifted(v_v, r0, i, c)):
                    acc = prob[w] * vw if acc is None else acc + prob[w] * vw
            o_v[pl.ds(half, RB // 2), i * LANES:(i + 1) * LANES] = _pack(acc)
            yield [acc]

    def attn_rows(r0, n_blocks):
        for b in range(n_blocks):
            start_row = r0 + b * RB
            if isinstance(r0, int):
                yield from attn_block(start_row, start_row // 2)
            else:
                yield from attn_block(pl.multiple_of(start_row, RB), pl.multiple_of(start_row // 2, RB // 2))

    slots = D // NP * (D // KP)
    zero = zero_s[0]

    def block_boundary():
        def body(_, carry):
            zero_s[0] = 0
            return carry
        lax.fori_loop(0, zero, body, 0)

    def chunk(r):
        return ("mod", r), ("mod", D + r), ("wq", r)

    def chunk_stages(r):
        sc_rows = jnp.broadcast_to(silu_c(), (MOD_ROWS, D))
        for lo in (r, D + r):
            m = jnp.dot(sc_rows, wmod_v[:, lo:lo + MA], preferred_element_type=F32)
            mod_v[:, lo:lo + MA] = m[0:8].astype(BF16).astype(F32)
        cols = slice(r, r + MA)
        h = _pack(x1_v[0:TA, cols] * (1.0 + mod_row(1)[:, cols]) + mod_row(0)[:, cols])
        ha_v[0:TA // 2, cols] = h
        yield []
        yield from permute_stages(0, r, r + MA)

    start(("x", 0), *chunk(0))
    wait(("x", 0))
    start(*chunk(MA))
    x1_v[0:TA, :] = _layernorm(x_v[0:TA, :].astype(F32))
    wait(*chunk(0))
    for _ in chunk_stages(0):
        pass
    for r in range(0, D, MA):
        if r + MA < D:
            wait(*chunk(r + MA))
            start(*(chunk(r + 2 * MA) if r + 2 * MA < D else (("x", 1), ("x", 2))))
            side = _Spread(chunk_stages(r + MA), 1 + MA // PR, D // LANES, never(zero))
        else:
            wait(("x", 1))
            start(*[("x", i) for i in range(3, n_a)], ("w", 1), ("w", 2))
            side = _Spread(ln_stages(x_v, ha_v, TA, TA, 0, 1), TA // LB, D // LANES, never(zero))
        nq = 4 * LANES * LANES // MA
        for lo in range(0, D, nq):
            parts = lane_tiles(jnp.dot(pltpu.bitcast(ha_v[0:TA // 2, r:r + MA], BF16),
                                       _load_bf16(wq_v, slice(r, r + MA), slice(lo, lo + nq)),
                                       preferred_element_type=F32))
            for j, part in enumerate(parts):
                cols = slice(lo + j * LANES, lo + (j + 1) * LANES)
                if r > 0:
                    part = q_v[0:TA, cols] + part
                q_v[0:TA, cols] = side.step(part)

    block_boundary()

    def next_ln(s):
        for _ in range(TA // LB):
            yield []
        wait(("x", s))
        if s == n_a - 1:
            start("wo", "mod_b")
        yield from ln_stages(x_v, ha_v, s * TA, TA, 0, 1)

    for s in range(1, n_a - 1):
        project(0, s, _Spread(next_ln(s + 1), 2 * (TA // LB), slots, never(zero)))
    wait(("w", 1))
    project(0, n_a - 1, _Spread(permute_stages(1), D // PR, slots, never(zero)))
    wait(("w", 2))
    project(1, 0, _Spread(permute_stages(2), D // PR, slots, never(zero)))
    wait("wo")
    project(1, 1, _Spread(wo_stages(), NT, slots, never(zero)))
    wait("mod_b")
    start("wg", "wu", "wd")
    side = _Spread(mod_b_stages(), 4 * D // LANES, (n_a - 2) * slots, never(zero))
    for s in range(2, n_a):
        project(1, s, side)
    first = TC // TA
    for s in range(first):
        project(2, s)
    k_v[0:HALO, :] = jnp.broadcast_to(k_v[HALO:HALO + 1, :], (HALO, D))
    v_v[0:HALO, :] = jnp.broadcast_to(v_v[HALO:HALO + 1, :], (HALO, D))
    side = _Spread(attn_rows(0, TC // RB), TC // RB * ATTN_STAGES, (n_a - first) * slots, never(zero))
    for s in range(first, n_a):
        project(2, s, side)
    wait("wg", "wu", "wd")

    def out_copy(t, slot, part):
        cols = pl.ds(part * OC, OC)
        return pltpu.make_async_copy(out_v.at[slot, :, cols], out_hbm.at[pl.ds(t * TC, TC), cols],
                                     out_sems.at[slot, part])

    n_c = S // TC

    def phase_c(t, carry):
        rows = pl.ds(pl.multiple_of(t * TC, TC), TC)
        slot = t % 2

        @pl.when(t >= 2)
        def _():
            for part in range(D // OC):
                out_copy(t - 2, slot, part).wait()
        for n, lo in enumerate(range(0, D, NP)):
            a = matmul_piece(o_v.at[pl.ds(pl.multiple_of(t * (TC // 2), TC // 2), TC // 2)], wo_v, lo, (accg_v, accu_v)[n % 2], None)
            x1_v[0:TC, lo:lo + NP] = x_v[rows, lo:lo + NP].astype(F32) + mod_row(2)[:, lo:lo + NP] * a
        h_v[...] = _pack(_layernorm(x1_v[0:TC, :]) * (1.0 + mod_row(4)) + mod_row(3))
        nxt = jnp.minimum(t + 1, n_c - 1) * TC
        n_slots = 3 * (F // NP) * (D // KP)
        side = _Spread(attn_rows(nxt, TC // RB), TC // RB * ATTN_STAGES, n_slots, never(nxt))
        for lo in range(0, F, NP):
            accg_v[...] = matmul_piece(h_v, wg_v, lo, accg_v, side)
            u = matmul_piece(h_v, wu_v, lo, accu_v, side)
            act_v[:, lo:lo + NP] = _pack(_silu(accg_v[...]) * u)
        for n, lo in enumerate(range(0, D, NP)):
            y = matmul_piece(act_v, wd_v, lo, (accg_v, accu_v)[n % 2], side)
            out_v[slot, :, lo:lo + NP] = (x1_v[0:TC, lo:lo + NP] + mod_row(5)[:, lo:lo + NP] * y).astype(BF16)
            if (lo + NP) % OC == 0:
                out_copy(t, slot, lo // OC).start()
        return carry
    lax.fori_loop(0, n_c, phase_c, 0)
    for t in range(n_c - 2, n_c):
        for part in range(D // OC):
            out_copy(t, t % 2, part).wait()


@jax.jit
def pallas_adaLN_cond__sliding_local_dilated__swiglu_ffn__prompt_kernel(
    A_x: jax.Array,
    A_wqkv: jax.Array,
    A_wo: jax.Array,
    B_x: jax.Array,
    B_w_gate: jax.Array,
    B_w_up: jax.Array,
    B_w_down: jax.Array,
    c: jax.Array,
    w_mod: jax.Array,
):
    del B_x
    hbm = pl.BlockSpec(memory_space=pl.ANY)
    out = pl.pallas_call(
        _kernel,
        out_shape=jax.ShapeDtypeStruct((S, D), BF16),
        in_specs=[hbm, hbm, hbm, hbm, hbm, hbm, pl.BlockSpec(memory_space=pltpu.VMEM), hbm],
        out_specs=hbm,
        scratch_shapes=[
            pltpu.VMEM((S, D), BF16),
            pltpu.VMEM((3, D, D), BF16),
            pltpu.VMEM((D // 2, D), U32),
            pltpu.VMEM((D // 2, D), U32),
            pltpu.VMEM((D // 2, D), U32),
            pltpu.VMEM((D, D), BF16),
            pltpu.VMEM((D // 2, D), U32),
            pltpu.VMEM((D, F), BF16),
            pltpu.VMEM((D, F), BF16),
            pltpu.VMEM((F, D), BF16),
            pltpu.VMEM((D, 6 * D), BF16),
            pltpu.VMEM((D, LANES), F32),
            pltpu.VMEM((8, 6 * D), F32),
            pltpu.VMEM((S, D), F32),
            pltpu.VMEM((S + HALO, D), F32),
            pltpu.VMEM((S + HALO, D), F32),
            pltpu.VMEM((S // 2, D), U32),
            pltpu.VMEM((TC // 2, F), U32),
            pltpu.VMEM((S // 2, D), U32),
            pltpu.VMEM((TC // 2, D), U32),
            pltpu.VMEM((max(TA, TC), D), F32),
            pltpu.VMEM((max(TA, TC), NP), F32),
            pltpu.VMEM((max(TA, TC), NP), F32),
            pltpu.VMEM((2, TC, D), BF16),
            pltpu.SMEM((1,), jnp.int32),
            pltpu.SemaphoreType.DMA((7 + S // TA + 3 * D // MA,)),
            pltpu.SemaphoreType.DMA((2, D // OC)),
        ],
        compiler_params=pltpu.CompilerParams(vmem_limit_bytes=120 * 1024 * 1024),
    )(A_x.reshape(S, D), A_wqkv, A_wo, B_w_gate, B_w_up, B_w_down, c, w_mod)
    return out.reshape(1, S, D)
```

```python
import jax
import jax.numpy as jnp
from jax import lax
from jax.experimental import pallas as pl
from jax.experimental.pallas import tpu as pltpu

S, D, F = 2048, 1024, 3584
H, DH, W, DIL = 32, 32, 8, 2
LANES = 128
NT = D // LANES
HALO = 16
TA = 512
RB = 32
TC = 512
NP, KP = 256, 512
PR = 64
LB = 32
MOD_ROWS, MA, MB = 16, 256, 32
OC = 256
ND1, DW = 3, 1
EPS = 1e-5
F32, BF16, U32 = jnp.float32, jnp.bfloat16, jnp.uint32


def _layernorm(x):
    m = jnp.mean(x, axis=-1, keepdims=True)
    xc = x - m
    v = jnp.mean(xc * xc, axis=-1, keepdims=True)
    return xc * lax.rsqrt(v + EPS)


def _silu(x):
    return x * (1.0 / (1.0 + jnp.exp(-x)))


ATTN_STAGES = W // 2 + 1 + NT


class _Spread:
    def __init__(self, gen, n_stages, n_slots, never, anchor):
        self.gen, self.n_stages, self.n_slots = gen, n_stages, n_slots
        self.never, self.anchor = never, anchor
        self.slot = self.done = 0
        self.pending = []

    def step(self, part):
        part, rest = part[:, :LANES], part[:, LANES:] if part.shape[1] > LANES else None
        if self.pending:
            tied = jnp.concatenate(self.pending, axis=0)
            for lo in range(0, tied.shape[0], part.shape[0]):
                n = min(part.shape[0], tied.shape[0] - lo)
                tail = jnp.where(self.never, tied[lo:lo + n], part[-n:])
                part = tail if n == part.shape[0] else jnp.concatenate([part[:-n], tail], axis=0)
        self.pending = []
        self.slot += 1
        while self.done < min(self.n_stages, self.n_stages * self.slot // (self.n_slots - 1)):
            self.anchor.append(part)
            self.pending += next(self.gen)
            self.anchor.pop()
            self.done += 1
        return part if rest is None else jnp.concatenate([part, rest], axis=1)


def _pack(x):
    return pltpu.bitcast(x.astype(BF16), U32)


def _load_bf16(ref, rows, cols):
    if ref.dtype == BF16:
        return ref[rows, cols]
    return pltpu.bitcast(ref[rows.start // 2:rows.stop // 2, cols], BF16)


def _kernel(x_hbm, wqkv_hbm, wo_hbm, wg_hbm, wu_hbm, wd_hbm, c_ref, wmod_hbm, zero_ref, out_hbm,
            x_v, wqkv_raw, wq_v, wk_v, wv_v, wo_raw, wo_v, wg_v, wu_v, wd_v, wmod_v, sc_v, mod_v,
            q_v, k_v, v_v, o_v, act_v, ha_v, h_v, x1_v, accg_v, accu_v, out_v, sems, out_sems):
    n_a = S // TA
    copies = {}

    def add_copy(name, src, dst):
        copies[name] = pltpu.make_async_copy(src, dst, sems.at[len(copies)])

    for r in range(0, D, MA):
        add_copy(("wq", r), wqkv_hbm.at[pl.ds(r, MA), pl.ds(0, D)], wqkv_raw.at[0, pl.ds(r, MA)])
    for p in (1, 2):
        add_copy(("w", p), wqkv_hbm.at[:, pl.ds(p * D, D)], wqkv_raw.at[p])
    for s in range(n_a):
        add_copy(("x", s), x_hbm.at[pl.ds(s * TA, TA)], x_v.at[pl.ds(s * TA, TA)])
    for lo in range(0, 2 * D, MA):
        add_copy(("mod", lo), wmod_hbm.at[:, pl.ds(lo, MA)], wmod_v.at[:, pl.ds(lo, MA)])
    add_copy("mod_b", wmod_hbm.at[:, pl.ds(2 * D, 4 * D)], wmod_v.at[:, pl.ds(2 * D, 4 * D)])
    add_copy("wo", wo_hbm, wo_raw)
    add_copy("wg", wg_hbm, wg_v)
    add_copy("wu", wu_hbm, wu_v)
    add_copy("wd", wd_hbm, wd_v)

    def start(*names):
        for name in names:
            copies[name].start()

    def wait(*names):
        for name in names:
            copies[name].wait()

    zero = zero_ref[0]
    never = lax.broadcasted_iota(jnp.int32, (1, LANES), 1) < zero
    anchor = []

    def spread(gen, n_stages, n_slots):
        return _Spread(gen, n_stages, n_slots, never, anchor)

    def after_anchor(x, i=0, n=1):
        if not anchor:
            return x
        lo = anchor[-1].shape[0] * i // n
        a = anchor[-1][lo:lo + x.shape[0]]
        return jnp.concatenate([jnp.where(never, a, x[:, j:j + LANES]) for j in range(0, x.shape[1], LANES)], axis=1)

    def block_boundary():
        def body(_, carry):
            mod_v[:, 0:LANES] = jnp.zeros((8, LANES), F32)
            return carry
        lax.fori_loop(0, zero, body, 0)

    def silu_c():
        return _silu(c_ref[...].astype(F32)).astype(BF16)

    def mod_row(i):
        return mod_v[0:1, i * D:(i + 1) * D]

    def mod_b_stages():
        sc = silu_c().astype(F32)
        for lo in range(0, D, LANES):
            sc_v[lo:lo + LANES, :] = jnp.broadcast_to(sc[:, lo:lo + LANES], (LANES, LANES)).T
        for lo in range(2 * D, 6 * D, LANES):
            acc = None
            for r in range(0, D, MB):
                part = wmod_v[r:r + MB, lo:lo + LANES].astype(F32) * sc_v[r:r + MB, :]
                if r % (4 * MB) == 0:
                    part = after_anchor(part, r, D)
                acc = part if acc is None else acc + part
            row = jnp.sum(acc, axis=0, keepdims=True).astype(BF16).astype(F32)
            row = jnp.broadcast_to(row, (8, LANES))
            mod_v[:, lo:lo + LANES] = row
            yield [row]

    def lane_tiles(v):
        return [v[:, j * LANES:(j + 1) * LANES] for j in range(v.shape[1] // LANES)]

    def ln_stages(src, dst, r0, n_rows, shift, scale):
        for r in range(r0, r0 + n_rows, LB):
            x = src[r:r + LB, :].astype(F32)
            x = jnp.concatenate([after_anchor(x[:, :LANES], r // LB % 2, 2), x[:, LANES:]], axis=1)
            h = _layernorm(x) * (1.0 + mod_row(scale)) + mod_row(shift)
            h = _pack(h)
            dst[r // 2:(r + LB) // 2, :] = h
            yield [pltpu.bitcast(t, F32) for t in lane_tiles(h)]

    def permute_rows_of(p, r):
        lane = lax.broadcasted_iota(jnp.int32, (PR // 2, LANES), 1)
        t = [_pack(wqkv_raw[p, pl.ds(2 * r, PR), j * LANES:(j + 1) * LANES]) for j in range(NT)]
        t[0] = pltpu.bitcast(after_anchor(pltpu.bitcast(t[0], F32)), U32)
        for b in range(3):
            sh = 4 << b
            low = (lane & sh) == 0
            for j in range(NT):
                if j & (1 << b):
                    continue
                lo_t, hi_t = t[j], t[j | (1 << b)]
                t[j] = jnp.where(low, lo_t, pltpu.roll(hi_t, sh, 1))
                t[j | (1 << b)] = jnp.where(low, pltpu.roll(lo_t, LANES - sh, 1), hi_t)
        for j in range(NT):
            (wq_v, wk_v, wv_v)[p][pl.ds(r, PR // 2), j * LANES:(j + 1) * LANES] = t[j]
        return [pltpu.bitcast(tj, F32) for tj in t]

    def permute_stages(p, lo=0, hi=D):
        for r in range(lo // 2, hi // 2, PR // 2):
            yield permute_rows_of(p, r)

    def wo_stages():
        for i in range(NT):
            done = []
            for hh in range(4):
                for jq in range(NT // 4):
                    pieces = []
                    for j in range(4 * jq, 4 * jq + 4):
                        src = (4 * j + hh) * DH + 4 * i
                        grp = wo_raw[src // 16 * 16:src // 16 * 16 + 16, :].astype(F32)
                        pieces.append(grp[src % 16:src % 16 + 4])
                    dst = i * LANES + hh * DH + jq * 16
                    blk = _pack(jnp.concatenate(pieces, axis=0))
                    wo_v[dst // 2:dst // 2 + 8, :] = blk
                    done += [pltpu.bitcast(t, F32) for t in lane_tiles(blk)]
            yield done

    def matmul_piece(lhs_ref, w_ref, lo, acc_ref, side):
        n_k = pl.cdiv(lhs_ref.shape[1], KP)
        for i in range(n_k):
            ks = slice(i * KP, min((i + 1) * KP, lhs_ref.shape[1]))
            part = jnp.dot(pltpu.bitcast(lhs_ref[:, ks], BF16), _load_bf16(w_ref, ks, slice(lo, lo + NP)),
                           preferred_element_type=F32)
            if i > 0:
                part = acc_ref[...] + part
            for sd in (side if isinstance(side, tuple) else () if side is None else (side,)):
                part = sd.step(part)
            if i == n_k - 1:
                return part
            acc_ref[...] = part

    def project(p, s, side=None):
        dst, off = ((q_v, 0), (k_v, HALO), (v_v, HALO))[p]
        r0 = s * TA
        for n, lo in enumerate(range(0, D, NP)):
            acc = (accg_v, accu_v)[n % 2].at[0:TA]
            dst[r0 + off:r0 + off + TA, lo:lo + NP] = matmul_piece(
                ha_v.at[r0 // 2:(r0 + TA) // 2], (wq_v, wk_v, wv_v)[p], lo, acc, side)

    lane_a = lax.broadcasted_iota(jnp.int32, (RB, LANES), 1)
    row_a = lax.broadcasted_iota(jnp.int32, (RB, LANES), 0)
    even1 = (lane_a & 1) == 0
    even2 = (lane_a & 2) == 0
    scale = DH ** -0.5

    def shifted(ref, r0, i, c, step, n_steps):
        win = after_anchor(ref[pl.ds(r0, RB + HALO), i * LANES:(i + 1) * LANES], step, n_steps)
        lo = HALO - 8 - DIL * c
        blk = win[lo:lo + RB + 8]
        return blk[8:], blk[:RB]

    def attn_block(r0, half):
        logit = [None] * W
        pos = row_a + r0
        for c in range(W // 2):
            ws = (c, c + W // 2)
            for i in range(NT):
                qi = q_v[pl.ds(r0, RB), i * LANES:(i + 1) * LANES]
                for w, kw in zip(ws, shifted(k_v, r0, i, c, i, NT)):
                    logit[w] = qi * kw if i == 0 else logit[w] + qi * kw
            for w in ws:
                s = logit[w]
                s = s + jnp.where(even1, pltpu.roll(s, LANES - 1, 1), pltpu.roll(s, 1, 1))
                s = s + jnp.where(even2, pltpu.roll(s, LANES - 2, 1), pltpu.roll(s, 2, 1))
                s = s * scale
                logit[w] = s if w == 0 else jnp.where(pos >= DIL * w, s, -1e9)
            yield [logit[w] for w in ws]
        m = logit[0]
        for w in range(1, W):
            m = jnp.maximum(m, logit[w])
        e = [jnp.exp(s - m) for s in logit]
        den = e[0]
        for w in range(1, W):
            den = den + e[w]
        inv = 1.0 / den
        prob = [ew * inv for ew in e]
        yield [inv]
        for i in range(NT):
            acc = None
            for c in range(W // 2):
                for w, vw in zip((c, c + W // 2), shifted(v_v, r0, i, c, c, W // 2)):
                    acc = prob[w] * vw if acc is None else acc + prob[w] * vw
            o_v[pl.ds(half, RB // 2), i * LANES:(i + 1) * LANES] = _pack(acc)
            yield [acc]

    def attn_rows(r0, n_blocks):
        for b in range(n_blocks):
            start_row = r0 + b * RB
            if isinstance(r0, int):
                yield from attn_block(start_row, start_row // 2)
            else:
                yield from attn_block(pl.multiple_of(start_row, RB), pl.multiple_of(start_row // 2, RB // 2))

    slots = D // NP * (D // KP)

    def chunk(r):
        return ("mod", r), ("mod", D + r), ("wq", r)

    def chunk_stages(r):
        sc_rows = jnp.broadcast_to(silu_c(), (MOD_ROWS, D))
        for lo in (r, D + r):
            m = jnp.dot(sc_rows, wmod_v[:, lo:lo + MA], preferred_element_type=F32)
            mod_v[:, lo:lo + MA] = m[0:8].astype(BF16).astype(F32)
        cols = slice(r, r + MA)
        h = _pack(x1_v[1, 0:TA, cols] * (1.0 + mod_row(1)[:, cols]) + mod_row(0)[:, cols])
        ha_v[0:TA // 2, cols] = h
        yield []
        yield from permute_stages(0, r, r + MA)

    start(("x", 0), *chunk(0))
    wait(("x", 0))
    start(*chunk(MA))
    x1_v[1, 0:TA, :] = _layernorm(x_v[0:TA, :].astype(F32))
    wait(*chunk(0))
    for _ in chunk_stages(0):
        pass
    for r in range(0, D, MA):
        if r + MA < D:
            wait(*chunk(r + MA))
            start(*(chunk(r + 2 * MA) if r + 2 * MA < D else (("x", 1), ("x", 2))))
            side = spread(chunk_stages(r + MA), 1 + MA // PR, D // LANES)
        else:
            wait(("x", 1))
            start(*[("x", i) for i in range(3, n_a)], ("w", 1), ("w", 2))
            side = spread(ln_stages(x_v, ha_v, TA, TA, 0, 1), TA // LB, D // LANES)
        nq = 4 * LANES * LANES // MA
        for lo in range(0, D, nq):
            parts = lane_tiles(jnp.dot(pltpu.bitcast(ha_v[0:TA // 2, r:r + MA], BF16),
                                       _load_bf16(wq_v, slice(r, r + MA), slice(lo, lo + nq)),
                                       preferred_element_type=F32))
            for j, part in enumerate(parts):
                cols = slice(lo + j * LANES, lo + (j + 1) * LANES)
                if r > 0:
                    part = q_v[0:TA, cols] + part
                q_v[0:TA, cols] = side.step(part)

    block_boundary()

    def next_ln(s):
        for _ in range(TA // LB):
            yield []
        wait(("x", s))
        if s == n_a - 1:
            start("wo", "mod_b")
        yield from ln_stages(x_v, ha_v, s * TA, TA, 0, 1)

    for s in range(1, n_a - 1):
        project(0, s, spread(next_ln(s + 1), 2 * (TA // LB), slots))
    wait(("w", 1))
    project(0, n_a - 1, spread(permute_stages(1), D // PR, slots))
    wait(("w", 2))
    project(1, 0, spread(permute_stages(2), D // PR, slots))
    wait("wo")
    project(1, 1, spread(wo_stages(), NT, slots))
    wait("mod_b")
    start("wg", "wu", "wd")
    side = spread(mod_b_stages(), 4 * D // LANES, (n_a - 2) * slots)
    for s in range(2, n_a):
        project(1, s, side)
    first = TC // TA
    for s in range(first):
        project(2, s)
    k_v[0:HALO, :] = jnp.broadcast_to(k_v[HALO:HALO + 1, :], (HALO, D))
    v_v[0:HALO, :] = jnp.broadcast_to(v_v[HALO:HALO + 1, :], (HALO, D))
    block_boundary()
    attn_stages = TC // RB * ATTN_STAGES
    side = spread(attn_rows(0, TC // RB), attn_stages, (n_a - 1 - first) * slots)
    for s in range(first, n_a - 1):
        project(2, s, side)

    def tile_rows(t, n):
        return slice(t * n, (t + 1) * n) if isinstance(t, int) else pl.ds(pl.multiple_of(t * n, n), n)

    def out_proj(t):
        for n, lo in enumerate(range(0, D, NP)):
            cols = slice(lo, lo + NP)
            a = matmul_piece(o_v.at[tile_rows(t, TC // 2)], wo_v, lo, (accg_v, accu_v)[n % 2], None)
            x1_v[t % 2, 0:TC, cols] = x_v[tile_rows(t, TC), cols].astype(F32) + mod_row(2)[:, cols] * a

    def ffn_norm(t, n_slots):
        return spread(ln_stages(x1_v.at[t % 2], h_v, 0, TC, 3, 4), TC // LB, n_slots)

    def out_copy(t, part):
        cols = pl.ds(part * OC, OC)
        return pltpu.make_async_copy(out_v.at[t % 2, :, cols], out_hbm.at[tile_rows(t, TC), cols],
                                     out_sems.at[t % 2, part])

    def out_wait(t):
        for part in range(D // OC):
            out_copy(t, part).wait()

    n_c = S // TC
    n_f = F // NP
    rounds = 2 * (D // KP)

    def down_piece(t, n, side):
        cols = slice(n * NP, (n + 1) * NP)
        y = matmul_piece(act_v, wd_v, n * NP, (accg_v, accu_v)[n % 2], side)
        out_v[t % 2, :, cols] = (x1_v[t % 2, 0:TC, cols] + mod_row(5)[:, cols] * y).astype(BF16)
        if cols.stop % OC == 0:
            out_copy(t, cols.start // OC).start()

    def phase_c(t, carry):
        @pl.when(t >= 2)
        def _():
            out_wait(t - 2)

        nxt = jnp.minimum(t + 1, n_c - 1)
        attn = spread(attn_rows(nxt * TC, TC // RB), attn_stages, n_f * rounds + DW * ND1 * pl.cdiv(F, KP))
        for lo in range(0, F, NP):
            accg_v[...] = matmul_piece(h_v, wg_v, lo, accg_v, attn)
            u = matmul_piece(h_v, wu_v, lo, accu_v, attn)
            act_v[:, lo:lo + NP] = _pack(_silu(accg_v[...]) * u)
        for n in range(ND1):
            down_piece(t, n, (attn,) * DW)

        @pl.when(t < n_c - 1)
        def _():
            out_proj(t + 1)

        norm = ffn_norm(t + 1, (D // NP - ND1) * pl.cdiv(F, KP))
        for n in range(ND1, D // NP):
            down_piece(t, n, norm)
        return carry

    out_proj(0)
    project(2, n_a - 1, ffn_norm(0, slots))
    wait("wg", "wu", "wd")
    lax.fori_loop(0, n_c, phase_c, 0)
    out_wait(n_c - 2)
    out_wait(n_c - 1)


@jax.jit
def pallas_adaLN_cond__sliding_local_dilated__swiglu_ffn__prompt_kernel(
    A_x: jax.Array,
    A_wqkv: jax.Array,
    A_wo: jax.Array,
    B_x: jax.Array,
    B_w_gate: jax.Array,
    B_w_up: jax.Array,
    B_w_down: jax.Array,
    c: jax.Array,
    w_mod: jax.Array,
):
    del B_x
    hbm = pl.BlockSpec(memory_space=pl.ANY)
    out = pl.pallas_call(
        _kernel,
        out_shape=jax.ShapeDtypeStruct((S, D), BF16),
        in_specs=[hbm, hbm, hbm, hbm, hbm, hbm, pl.BlockSpec(memory_space=pltpu.VMEM), hbm,
                  pl.BlockSpec(memory_space=pltpu.SMEM)],
        out_specs=hbm,
        scratch_shapes=[
            pltpu.VMEM((S, D), BF16),
            pltpu.VMEM((3, D, D), BF16),
            pltpu.VMEM((D // 2, D), U32),
            pltpu.VMEM((D // 2, D), U32),
            pltpu.VMEM((D // 2, D), U32),
            pltpu.VMEM((D, D), BF16),
            pltpu.VMEM((D // 2, D), U32),
            pltpu.VMEM((D, F), BF16),
            pltpu.VMEM((D, F), BF16),
            pltpu.VMEM((F, D), BF16),
            pltpu.VMEM((D, 6 * D), BF16),
            pltpu.VMEM((D, LANES), F32),
            pltpu.VMEM((8, 6 * D), F32),
            pltpu.VMEM((S, D), F32),
            pltpu.VMEM((S + HALO, D), F32),
            pltpu.VMEM((S + HALO, D), F32),
            pltpu.VMEM((S // 2, D), U32),
            pltpu.VMEM((TC // 2, F), U32),
            pltpu.VMEM((S // 2, D), U32),
            pltpu.VMEM((TC // 2, D), U32),
            pltpu.VMEM((2, max(TA, TC), D), F32),
            pltpu.VMEM((max(TA, TC), NP), F32),
            pltpu.VMEM((max(TA, TC), NP), F32),
            pltpu.VMEM((2, TC, D), BF16),
            pltpu.SemaphoreType.DMA((7 + S // TA + 3 * D // MA,)),
            pltpu.SemaphoreType.DMA((2, D // OC)),
        ],
        compiler_params=pltpu.CompilerParams(vmem_limit_bytes=120 * 1024 * 1024),
    )(A_x.reshape(S, D), A_wqkv, A_wo, B_w_gate, B_w_up, B_w_down, c, w_mod, jnp.zeros((1,), jnp.int32))
    return out.reshape(1, S, D)
```

```python
import jax
import jax.numpy as jnp
from jax import lax
from jax.experimental import pallas as pl
from jax.experimental.pallas import tpu as pltpu

S, D, F = 2048, 1024, 3584
H, DH, W, DIL = 32, 32, 8, 2
LANES = 128
NT = D // LANES
HALO = 16
TA = 512
RB = 32
TC = 512
NP, KP = 256, 512
PR = 64
LB = 64
MOD_ROWS, MA, MB = 16, 256, 32
OC = 256
ND1, DW = 3, 1
MT = 1
EPS = 1e-5
assert TA == TC
F32, BF16, U32 = jnp.float32, jnp.bfloat16, jnp.uint32


def _layernorm(x):
    m = jnp.mean(x, axis=-1, keepdims=True)
    xc = x - m
    v = jnp.mean(xc * xc, axis=-1, keepdims=True)
    return xc * lax.rsqrt(v + EPS)


def _silu(x):
    return x * (1.0 / (1.0 + jnp.exp(-x)))


ATTN_STAGES = W // 2 + 1 + NT


class _Spread:
    def __init__(self, gen, n_stages, n_slots, never, anchor):
        self.gen, self.n_stages, self.n_slots = gen, n_stages, n_slots
        self.never, self.anchor = never, anchor
        self.slot = self.done = 0
        self.pending = []

    def step(self, part):
        part, rest = part[:, :LANES], part[:, LANES:] if part.shape[1] > LANES else None
        if self.pending:
            tied = jnp.concatenate(self.pending, axis=0)
            for lo in range(0, tied.shape[0], part.shape[0]):
                n = min(part.shape[0], tied.shape[0] - lo)
                tail = jnp.where(self.never, tied[lo:lo + n], part[-n:])
                part = tail if n == part.shape[0] else jnp.concatenate([part[:-n], tail], axis=0)
        self.pending = []
        self.slot += 1
        while self.done < min(self.n_stages, self.n_stages * self.slot // (self.n_slots - 1)):
            self.anchor.append(part)
            self.pending += next(self.gen)
            self.anchor.pop()
            self.done += 1
        return part if rest is None else jnp.concatenate([part, rest], axis=1)


def _pack(x):
    return pltpu.bitcast(x.astype(BF16), U32)


def _load_bf16(ref, rows, cols):
    if ref.dtype == BF16:
        return ref[rows, cols]
    return pltpu.bitcast(ref[rows.start // 2:rows.stop // 2, cols], BF16)


def _kernel(x_hbm, wqkv_hbm, wo_hbm, wg_hbm, wu_hbm, wd_hbm, c_ref, wmod_hbm, zero_ref, out_hbm,
            x_v, wqkv_raw, wq_v, wk_v, wv_v, wo_raw, wo_v, wg_v, wu_v, wd_v, wmod_v, sc_v, mod_v,
            q_v, k_v, v_v, o_v, act_v, ha_v, h_v, x1_v, accg_v, accu_v, out_v, sems, out_sems):
    n_a = S // TA
    copies = {}

    def add_copy(name, src, dst):
        copies[name] = pltpu.make_async_copy(src, dst, sems.at[len(copies)])

    for r in range(0, D, MA):
        add_copy(("wq", r), wqkv_hbm.at[pl.ds(r, MA), pl.ds(0, D)], wqkv_raw.at[0, pl.ds(r, MA)])
    for p in (1, 2):
        add_copy(("w", p), wqkv_hbm.at[:, pl.ds(p * D, D)], wqkv_raw.at[p])
    for s in range(n_a):
        add_copy(("x", s), x_hbm.at[pl.ds(s * TA, TA)], x_v.at[pl.ds(s * TA, TA)])
    for lo in range(0, 2 * D, MA):
        add_copy(("mod", lo), wmod_hbm.at[:, pl.ds(lo, MA)], wmod_v.at[:, pl.ds(lo, MA)])
    add_copy("mod_b", wmod_hbm.at[:, pl.ds(2 * D, 4 * D)], wmod_v.at[:, pl.ds(2 * D, 4 * D)])
    add_copy("wo", wo_hbm, wo_raw)
    add_copy("wg", wg_hbm, wg_v)
    add_copy("wu", wu_hbm, wu_v)
    add_copy("wd", wd_hbm, wd_v)

    def start(*names):
        for name in names:
            copies[name].start()

    def wait(*names):
        for name in names:
            copies[name].wait()

    never = lax.broadcasted_iota(jnp.int32, (1, LANES), 1) < zero_ref[0]
    anchor = []

    def spread(gen, n_stages, n_slots):
        return _Spread(gen, n_stages, n_slots, never, anchor)

    def after_anchor(x, i=0, n=1):
        if not anchor:
            return x
        lo = anchor[-1].shape[0] * i // n
        a = anchor[-1][lo:lo + x.shape[0]]
        return jnp.concatenate([jnp.where(never, a, x[:, j:j + LANES]) for j in range(0, x.shape[1], LANES)], axis=1)

    def silu_c():
        return _silu(c_ref[...].astype(F32)).astype(BF16)

    def mod_row(i):
        return mod_v[0:1, i * D:(i + 1) * D]

    def mod_b_stages():
        sc = silu_c().astype(F32)
        for lo in range(0, D, LANES):
            sc_v[lo:lo + LANES, :] = jnp.broadcast_to(sc[:, lo:lo + LANES], (LANES, LANES)).T
        for lo in range(2 * D, 6 * D, LANES):
            acc = None
            for r in range(0, D, MB):
                part = wmod_v[r:r + MB, lo:lo + LANES].astype(F32) * sc_v[r:r + MB, :]
                if r % (4 * MB) == 0:
                    part = after_anchor(part, r, D)
                acc = part if acc is None else acc + part
            row = jnp.sum(acc, axis=0, keepdims=True).astype(BF16).astype(F32)
            row = jnp.broadcast_to(row, (8, LANES))
            mod_v[:, lo:lo + LANES] = row
            yield [row]

    def lane_tiles(v):
        return [v[:, j * LANES:(j + 1) * LANES] for j in range(v.shape[1] // LANES)]

    def ln_stages(src, dst, r0, n_rows, shift, scale):
        for r in range(r0, r0 + n_rows, LB):
            x = src[r:r + LB, :].astype(F32)
            x = jnp.concatenate([after_anchor(x[:, :LANES], r // LB % 2, 2), x[:, LANES:]], axis=1)
            h = _layernorm(x) * (1.0 + mod_row(scale)) + mod_row(shift)
            h = _pack(h)
            dst[r // 2:(r + LB) // 2, :] = h
            yield [pltpu.bitcast(t, F32) for t in lane_tiles(h)]

    def permute_rows_of(p, r):
        lane = lax.broadcasted_iota(jnp.int32, (PR // 2, LANES), 1)
        t = [_pack(wqkv_raw[p, pl.ds(2 * r, PR), j * LANES:(j + 1) * LANES]) for j in range(NT)]
        t[0] = pltpu.bitcast(after_anchor(pltpu.bitcast(t[0], F32)), U32)
        for b in range(3):
            sh = 4 << b
            low = (lane & sh) == 0
            for j in range(NT):
                if j & (1 << b):
                    continue
                lo_t, hi_t = t[j], t[j | (1 << b)]
                t[j] = jnp.where(low, lo_t, pltpu.roll(hi_t, sh, 1))
                t[j | (1 << b)] = jnp.where(low, pltpu.roll(lo_t, LANES - sh, 1), hi_t)
        for j in range(NT):
            (wq_v, wk_v, wv_v)[p][pl.ds(r, PR // 2), j * LANES:(j + 1) * LANES] = t[j]
        return [pltpu.bitcast(tj, F32) for tj in t]

    def permute_stages(p, lo=0, hi=D):
        for r in range(lo // 2, hi // 2, PR // 2):
            yield permute_rows_of(p, r)

    def wo_stages():
        for i in range(NT):
            done = []
            for hh in range(4):
                for jq in range(NT // 4):
                    pieces = []
                    for j in range(4 * jq, 4 * jq + 4):
                        src = (4 * j + hh) * DH + 4 * i
                        grp = wo_raw[src // 16 * 16:src // 16 * 16 + 16, :].astype(F32)
                        pieces.append(grp[src % 16:src % 16 + 4])
                    dst = i * LANES + hh * DH + jq * 16
                    blk = _pack(jnp.concatenate(pieces, axis=0))
                    wo_v[dst // 2:dst // 2 + 8, :] = blk
                    done += [pltpu.bitcast(t, F32) for t in lane_tiles(blk)]
            yield done

    def matmul_piece(lhs_ref, w_ref, lo, acc_ref, side):
        n_k = pl.cdiv(lhs_ref.shape[1], KP)
        for i in range(n_k):
            ks = slice(i * KP, min((i + 1) * KP, lhs_ref.shape[1]))
            part = jnp.dot(pltpu.bitcast(lhs_ref[:, ks], BF16), _load_bf16(w_ref, ks, slice(lo, lo + NP)),
                           preferred_element_type=F32)
            if i > 0:
                part = acc_ref[...] + part
            for sd in (side if isinstance(side, tuple) else () if side is None else (side,)):
                part = sd.step(part)
            if i == n_k - 1:
                return part
            acc_ref[...] = part

    def project(p, s, side=None):
        dst, off = ((q_v, 0), (k_v, HALO), (v_v, HALO))[p]
        r0 = s * TA
        for n, lo in enumerate(range(0, D, NP)):
            acc = (accg_v, accu_v)[n % 2].at[0:TA]
            dst[r0 + off:r0 + off + TA, lo:lo + NP] = matmul_piece(
                ha_v.at[r0 // 2:(r0 + TA) // 2], (wq_v, wk_v, wv_v)[p], lo, acc, side)

    lane_a = lax.broadcasted_iota(jnp.int32, (RB, LANES), 1)
    row_a = lax.broadcasted_iota(jnp.int32, (RB, LANES), 0)
    even1 = (lane_a & 1) == 0
    even2 = (lane_a & 2) == 0
    scale = DH ** -0.5

    def shifted(ref, r0, i, c, step, n_steps):
        win = after_anchor(ref[pl.ds(r0, RB + HALO), i * LANES:(i + 1) * LANES], step, n_steps)
        lo = HALO - 8 - DIL * c
        blk = win[lo:lo + RB + 8]
        return blk[8:], blk[:RB]

    def attn_block(r0, half):
        logit = [None] * W
        pos = row_a + r0
        for c in range(W // 2):
            ws = (c, c + W // 2)
            for i in range(NT):
                qi = q_v[pl.ds(r0, RB), i * LANES:(i + 1) * LANES]
                for w, kw in zip(ws, shifted(k_v, r0, i, c, i, NT)):
                    logit[w] = qi * kw if i == 0 else logit[w] + qi * kw
            for w in ws:
                s = logit[w]
                s = s + jnp.where(even1, pltpu.roll(s, LANES - 1, 1), pltpu.roll(s, 1, 1))
                s = s + jnp.where(even2, pltpu.roll(s, LANES - 2, 1), pltpu.roll(s, 2, 1))
                s = s * scale
                logit[w] = s if w == 0 else jnp.where(pos >= DIL * w, s, -1e9)
            yield [logit[w] for w in ws]
        m = logit[0]
        for w in range(1, W):
            m = jnp.maximum(m, logit[w])
        e = [jnp.exp(s - m) for s in logit]
        den = e[0]
        for w in range(1, W):
            den = den + e[w]
        inv = 1.0 / den
        prob = [ew * inv for ew in e]
        yield [inv]
        for i in range(NT):
            acc = None
            for c in range(W // 2):
                for w, vw in zip((c, c + W // 2), shifted(v_v, r0, i, c, c, W // 2)):
                    acc = prob[w] * vw if acc is None else acc + prob[w] * vw
            o_v[pl.ds(half, RB // 2), i * LANES:(i + 1) * LANES] = _pack(acc)
            yield [acc]

    def attn_rows(r0, n_blocks):
        for b in range(n_blocks):
            start_row = r0 + b * RB
            if isinstance(r0, int):
                yield from attn_block(start_row, start_row // 2)
            else:
                yield from attn_block(pl.multiple_of(start_row, RB), pl.multiple_of(start_row // 2, RB // 2))

    slots = D // NP * (D // KP)

    def chunk(r):
        return ("mod", r), ("mod", D + r), ("wq", r)

    def chunk_stages(r):
        sc_rows = jnp.broadcast_to(silu_c(), (MOD_ROWS, D))
        for lo in (r, D + r):
            m = jnp.dot(sc_rows, wmod_v[:, lo:lo + MA], preferred_element_type=F32)
            mod_v[:, lo:lo + MA] = m[0:8].astype(BF16).astype(F32)
        cols = slice(r, r + MA)
        h = _pack(x1_v[1, 0:TA, cols] * (1.0 + mod_row(1)[:, cols]) + mod_row(0)[:, cols])
        ha_v[0:TA // 2, cols] = h
        yield []
        yield from permute_stages(0, r, r + MA)

    start(("x", 0), *chunk(0))
    wait(("x", 0))
    start(*chunk(MA))
    x1_v[1, 0:TA, :] = _layernorm(x_v[0:TA, :].astype(F32))
    wait(*chunk(0))
    for _ in chunk_stages(0):
        pass
    for r in range(0, D, MA):
        if r + MA < D:
            wait(*chunk(r + MA))
            start(*(chunk(r + 2 * MA) if r + 2 * MA < D else (("x", 1), ("x", 2))))
            side = spread(chunk_stages(r + MA), 1 + MA // PR, D // LANES)
        else:
            wait(("x", 1))
            start(*[("x", i) for i in range(3, n_a)], ("w", 1), ("w", 2))
            side = spread(ln_stages(x_v, ha_v, TA, TA, 0, 1), TA // LB, D // LANES)
        nq = 4 * LANES * LANES // MA
        for lo in range(0, D, nq):
            parts = lane_tiles(jnp.dot(pltpu.bitcast(ha_v[0:TA // 2, r:r + MA], BF16),
                                       _load_bf16(wq_v, slice(r, r + MA), slice(lo, lo + nq)),
                                       preferred_element_type=F32))
            for j, part in enumerate(parts):
                cols = slice(lo + j * LANES, lo + (j + 1) * LANES)
                if r > 0:
                    part = q_v[0:TA, cols] + part
                q_v[0:TA, cols] = side.step(part)

    def next_ln(s):
        for _ in range(TA // LB):
            yield []
        wait(("x", s))
        if s == n_a - 1:
            start("wo", "mod_b")
        yield from ln_stages(x_v, ha_v, s * TA, TA, 0, 1)

    for s in range(1, n_a - 1):
        project(0, s, spread(next_ln(s + 1), 2 * (TA // LB), slots))
    wait(("w", 1))
    project(0, n_a - 1, spread(permute_stages(1), D // PR, slots))
    wait(("w", 2))
    project(1, 0, spread(permute_stages(2), D // PR, slots))
    wait("wo")
    project(2, 0, spread(wo_stages(), NT, slots))
    k_v[0:HALO, :] = jnp.broadcast_to(k_v[HALO:HALO + 1, :], (HALO, D))
    v_v[0:HALO, :] = jnp.broadcast_to(v_v[HALO:HALO + 1, :], (HALO, D))
    wait("mod_b")
    start("wg", "wu", "wd")
    attn_stages = TC // RB * ATTN_STAGES
    rest = [(p, s) for s in range(1, n_a) for p in (1, 2)][:-1]
    n_mod = MT * slots
    side = (spread(mod_b_stages(), 4 * D // LANES, n_mod),
            spread(attn_rows(0, TC // RB), attn_stages, len(rest) * slots - n_mod))
    for n, (p, s) in enumerate(rest):
        project(p, s, side[n >= MT])

    def tile_rows(t, n):
        return slice(t * n, (t + 1) * n) if isinstance(t, int) else pl.ds(pl.multiple_of(t * n, n), n)

    def out_proj(t):
        for n, lo in enumerate(range(0, D, NP)):
            cols = slice(lo, lo + NP)
            a = matmul_piece(o_v.at[tile_rows(t, TC // 2)], wo_v, lo, (accg_v, accu_v)[n % 2], None)
            x1_v[t % 2, 0:TC, cols] = x_v[tile_rows(t, TC), cols].astype(F32) + mod_row(2)[:, cols] * a

    def ffn_norm(t, n_slots):
        return spread(ln_stages(x1_v.at[t % 2], h_v, 0, TC, 3, 4), TC // LB, n_slots)

    def out_copy(t, part):
        cols = pl.ds(part * OC, OC)
        return pltpu.make_async_copy(out_v.at[t % 2, :, cols], out_hbm.at[tile_rows(t, TC), cols],
                                     out_sems.at[t % 2, part])

    def out_wait(t):
        for part in range(D // OC):
            out_copy(t, part).wait()

    n_c = S // TC
    n_f = F // NP
    rounds = 2 * (D // KP)

    def down_piece(t, n, side):
        cols = slice(n * NP, (n + 1) * NP)
        y = matmul_piece(act_v, wd_v, n * NP, (accg_v, accu_v)[n % 2], side)
        out_v[t % 2, :, cols] = (x1_v[t % 2, 0:TC, cols] + mod_row(5)[:, cols] * y).astype(BF16)
        if cols.stop % OC == 0:
            out_copy(t, cols.start // OC).start()

    def phase_c(t, carry):
        @pl.when(t >= 2)
        def _():
            out_wait(t - 2)

        nxt = jnp.minimum(t + 1, n_c - 1)
        attn = spread(attn_rows(nxt * TC, TC // RB), attn_stages, n_f * rounds + DW * ND1 * pl.cdiv(F, KP))
        for lo in range(0, F, NP):
            accg_v[...] = matmul_piece(h_v, wg_v, lo, accg_v, attn)
            u = matmul_piece(h_v, wu_v, lo, accu_v, attn)
            act_v[:, lo:lo + NP] = _pack(_silu(accg_v[...]) * u)
        for n in range(ND1):
            down_piece(t, n, (attn,) * DW)

        @pl.when(t < n_c - 1)
        def _():
            out_proj(t + 1)

        norm = ffn_norm(t + 1, (D // NP - ND1) * pl.cdiv(F, KP))
        for n in range(ND1, D // NP):
            down_piece(t, n, norm)
        return carry

    out_proj(0)
    project(2, n_a - 1, ffn_norm(0, slots))
    wait("wg", "wu", "wd")
    lax.fori_loop(0, n_c, phase_c, 0)
    out_wait(n_c - 2)
    out_wait(n_c - 1)


@jax.jit
def pallas_adaLN_cond__sliding_local_dilated__swiglu_ffn__prompt_kernel(
    A_x: jax.Array,
    A_wqkv: jax.Array,
    A_wo: jax.Array,
    B_x: jax.Array,
    B_w_gate: jax.Array,
    B_w_up: jax.Array,
    B_w_down: jax.Array,
    c: jax.Array,
    w_mod: jax.Array,
):
    del B_x
    hbm = pl.BlockSpec(memory_space=pl.ANY)
    out = pl.pallas_call(
        _kernel,
        out_shape=jax.ShapeDtypeStruct((S, D), BF16),
        in_specs=[hbm, hbm, hbm, hbm, hbm, hbm, pl.BlockSpec(memory_space=pltpu.VMEM), hbm,
                  pl.BlockSpec(memory_space=pltpu.SMEM)],
        out_specs=hbm,
        scratch_shapes=[
            pltpu.VMEM((S, D), BF16),
            pltpu.VMEM((3, D, D), BF16),
            pltpu.VMEM((D // 2, D), U32),
            pltpu.VMEM((D // 2, D), U32),
            pltpu.VMEM((D // 2, D), U32),
            pltpu.VMEM((D, D), BF16),
            pltpu.VMEM((D // 2, D), U32),
            pltpu.VMEM((D, F), BF16),
            pltpu.VMEM((D, F), BF16),
            pltpu.VMEM((F, D), BF16),
            pltpu.VMEM((D, 6 * D), BF16),
            pltpu.VMEM((D, LANES), F32),
            pltpu.VMEM((8, 6 * D), F32),
            pltpu.VMEM((S, D), F32),
            pltpu.VMEM((S + HALO, D), F32),
            pltpu.VMEM((S + HALO, D), F32),
            pltpu.VMEM((S // 2, D), U32),
            pltpu.VMEM((TC // 2, F), U32),
            pltpu.VMEM((S // 2, D), U32),
            pltpu.VMEM((TC // 2, D), U32),
            pltpu.VMEM((2, max(TA, TC), D), F32),
            pltpu.VMEM((max(TA, TC), NP), F32),
            pltpu.VMEM((max(TA, TC), NP), F32),
            pltpu.VMEM((2, TC, D), BF16),
            pltpu.SemaphoreType.DMA((7 + S // TA + 3 * D // MA,)),
            pltpu.SemaphoreType.DMA((2, D // OC)),
        ],
        compiler_params=pltpu.CompilerParams(vmem_limit_bytes=120 * 1024 * 1024),
    )(A_x.reshape(S, D), A_wqkv, A_wo, B_w_gate, B_w_up, B_w_down, c, w_mod, jnp.zeros((1,), jnp.int32))
    return out.reshape(1, S, D)
```

```python
import jax
import jax.numpy as jnp
from jax import lax
from jax.experimental import pallas as pl
from jax.experimental.pallas import tpu as pltpu

S, D, F = 2048, 1024, 3584
H, DH, W, DIL = 32, 32, 8, 2
LANES = 128
NT = D // LANES
HALO = 16
TA = 512
RB = 32
TC = 512
NP, KP = 256, 512
PR = 64
LB = 64
MOD_ROWS, MA, MB = 16, 256, 32
OC = 256
ND1, DW = 3, 1
MT = 1
EPS = 1e-5
assert TA == TC
F32, BF16, U32 = jnp.float32, jnp.bfloat16, jnp.uint32


def _layernorm(x):
    m = jnp.mean(x, axis=-1, keepdims=True)
    xc = x - m
    v = jnp.mean(xc * xc, axis=-1, keepdims=True)
    return xc * lax.rsqrt(v + EPS)


def _silu(x):
    return x * (1.0 / (1.0 + jnp.exp(-x)))


ATTN_STAGES = W // 2 + 1 + NT


class _Spread:
    def __init__(self, gen, n_stages, n_slots, never, anchor):
        self.gen, self.n_stages, self.n_slots = gen, n_stages, n_slots
        self.never, self.anchor = never, anchor
        self.slot = self.done = 0
        self.pending = []

    def step(self, part):
        part, rest = part[:, :LANES], part[:, LANES:] if part.shape[1] > LANES else None
        if self.pending:
            tied = jnp.concatenate(self.pending, axis=0)
            for lo in range(0, tied.shape[0], part.shape[0]):
                n = min(part.shape[0], tied.shape[0] - lo)
                tail = jnp.where(self.never, tied[lo:lo + n], part[-n:])
                part = tail if n == part.shape[0] else jnp.concatenate([part[:-n], tail], axis=0)
        self.pending = []
        self.slot += 1
        while self.done < min(self.n_stages, self.n_stages * self.slot // (self.n_slots - 1)):
            self.anchor.append(part)
            self.pending += next(self.gen)
            self.anchor.pop()
            self.done += 1
        return part if rest is None else jnp.concatenate([part, rest], axis=1)


def _pack(x):
    return pltpu.bitcast(x.astype(BF16), U32)


def _load_bf16(ref, rows, cols):
    if ref.dtype == BF16:
        return ref[rows, cols]
    return pltpu.bitcast(ref[rows.start // 2:rows.stop // 2, cols], BF16)


def _kernel(x_hbm, wqkv_hbm, wo_hbm, wg_hbm, wu_hbm, wd_hbm, c_ref, wmod_hbm, zero_ref, out_hbm,
            x_v, wqkv_raw, wq_v, wk_v, wv_v, wo_raw, wo_v, wg_v, wu_v, wd_v, wmod_v, sc_v, mod_v,
            q_v, k_v, v_v, o_v, act_v, ha_v, h_v, x1_v, accg_v, accu_v, out_v, sems, out_sems):
    n_a = S // TA
    copies = {}

    def add_copy(name, src, dst):
        copies[name] = pltpu.make_async_copy(src, dst, sems.at[len(copies)])

    for r in range(0, D, MA):
        add_copy(("wq", r), wqkv_hbm.at[pl.ds(r, MA), pl.ds(0, D)], wqkv_raw.at[0, pl.ds(r, MA)])
    for p in (1, 2):
        add_copy(("w", p), wqkv_hbm.at[:, pl.ds(p * D, D)], wqkv_raw.at[p])
    for s in range(n_a):
        add_copy(("x", s), x_hbm.at[pl.ds(s * TA, TA)], x_v.at[pl.ds(s * TA, TA)])
    for lo in range(0, 2 * D, MA):
        add_copy(("mod", lo), wmod_hbm.at[:, pl.ds(lo, MA)], wmod_v.at[:, pl.ds(lo, MA)])
    add_copy("mod_b", wmod_hbm.at[:, pl.ds(2 * D, 4 * D)], wmod_v.at[:, pl.ds(2 * D, 4 * D)])
    add_copy("wo", wo_hbm, wo_raw)
    add_copy("wg", wg_hbm, wg_v)
    add_copy("wu", wu_hbm, wu_v)
    add_copy("wd", wd_hbm, wd_v)

    def start(*names):
        for name in names:
            copies[name].start()

    def wait(*names):
        for name in names:
            copies[name].wait()

    never = lax.broadcasted_iota(jnp.int32, (1, LANES), 1) < zero_ref[0]
    anchor = []

    def spread(gen, n_stages, n_slots):
        return _Spread(gen, n_stages, n_slots, never, anchor)

    def after_anchor(x, i=0, n=1):
        if not anchor:
            return x
        lo = anchor[-1].shape[0] * i // n
        a = anchor[-1][lo:lo + x.shape[0]]
        return jnp.concatenate([jnp.where(never, a, x[:, j:j + LANES]) for j in range(0, x.shape[1], LANES)], axis=1)

    def silu_c():
        return _silu(c_ref[...].astype(F32)).astype(BF16)

    def mod_row(i):
        return mod_v[0:1, i * D:(i + 1) * D]

    def mod_b_stages():
        sc = silu_c().astype(F32)
        for lo in range(0, D, LANES):
            sc_v[lo:lo + LANES, :] = jnp.broadcast_to(sc[:, lo:lo + LANES], (LANES, LANES)).T
        for lo in range(2 * D, 6 * D, LANES):
            acc = None
            for r in range(0, D, MB):
                part = wmod_v[r:r + MB, lo:lo + LANES].astype(F32) * sc_v[r:r + MB, :]
                if r % (4 * MB) == 0:
                    part = after_anchor(part, r, D)
                acc = part if acc is None else acc + part
            row = jnp.sum(acc, axis=0, keepdims=True).astype(BF16).astype(F32)
            row = jnp.broadcast_to(row, (8, LANES))
            mod_v[:, lo:lo + LANES] = row
            yield [row]

    def lane_tiles(v):
        return [v[:, j * LANES:(j + 1) * LANES] for j in range(v.shape[1] // LANES)]

    def ln_stages(src, dst, r0, n_rows, shift, scale):
        for r in range(r0, r0 + n_rows, LB):
            x = src[r:r + LB, :].astype(F32)
            x = jnp.concatenate([after_anchor(x[:, :LANES], r // LB % 2, 2), x[:, LANES:]], axis=1)
            h = _layernorm(x) * (1.0 + mod_row(scale)) + mod_row(shift)
            h = _pack(h)
            dst[r // 2:(r + LB) // 2, :] = h
            yield [pltpu.bitcast(t, F32) for t in lane_tiles(h)]

    def permute_rows_of(p, r):
        lane = lax.broadcasted_iota(jnp.int32, (PR // 2, LANES), 1)
        t = [_pack(wqkv_raw[p, pl.ds(2 * r, PR), j * LANES:(j + 1) * LANES]) for j in range(NT)]
        t[0] = pltpu.bitcast(after_anchor(pltpu.bitcast(t[0], F32)), U32)
        for b in range(3):
            sh = 4 << b
            low = (lane & sh) == 0
            for j in range(NT):
                if j & (1 << b):
                    continue
                lo_t, hi_t = t[j], t[j | (1 << b)]
                t[j] = jnp.where(low, lo_t, pltpu.roll(hi_t, sh, 1))
                t[j | (1 << b)] = jnp.where(low, pltpu.roll(lo_t, LANES - sh, 1), hi_t)
        for j in range(NT):
            (wq_v, wk_v, wv_v)[p][pl.ds(r, PR // 2), j * LANES:(j + 1) * LANES] = t[j]
        return [pltpu.bitcast(tj, F32) for tj in t]

    def permute_stages(p, lo=0, hi=D):
        for r in range(lo // 2, hi // 2, PR // 2):
            yield permute_rows_of(p, r)

    def wo_stages():
        for i in range(NT):
            done = []
            for hh in range(4):
                for jq in range(NT // 4):
                    pieces = []
                    for j in range(4 * jq, 4 * jq + 4):
                        src = (4 * j + hh) * DH + 4 * i
                        grp = wo_raw[src // 16 * 16:src // 16 * 16 + 16, :].astype(F32)
                        pieces.append(grp[src % 16:src % 16 + 4])
                    dst = i * LANES + hh * DH + jq * 16
                    blk = _pack(jnp.concatenate(pieces, axis=0))
                    wo_v[dst // 2:dst // 2 + 8, :] = blk
                    done += [pltpu.bitcast(t, F32) for t in lane_tiles(blk)]
            yield done

    def matmul_piece(lhs_ref, w_ref, lo, acc_ref, side):
        n_k = pl.cdiv(lhs_ref.shape[1], KP)
        for i in range(n_k):
            ks = slice(i * KP, min((i + 1) * KP, lhs_ref.shape[1]))
            part = jnp.dot(pltpu.bitcast(lhs_ref[:, ks], BF16), _load_bf16(w_ref, ks, slice(lo, lo + NP)),
                           preferred_element_type=F32)
            if i > 0:
                part = acc_ref[...] + part
            for sd in (side if isinstance(side, tuple) else () if side is None else (side,)):
                part = sd.step(part)
            if i == n_k - 1:
                return part
            acc_ref[...] = part

    def project(p, s, side=None):
        dst, off = ((q_v, 0), (k_v, HALO), (v_v, HALO))[p]
        r0 = s * TA
        for n, lo in enumerate(range(0, D, NP)):
            acc = (accg_v, accu_v)[n % 2].at[0:TA]
            dst[r0 + off:r0 + off + TA, lo:lo + NP] = matmul_piece(
                ha_v.at[r0 // 2:(r0 + TA) // 2], (wq_v, wk_v, wv_v)[p], lo, acc, side)

    lane_a = lax.broadcasted_iota(jnp.int32, (RB, LANES), 1)
    row_a = lax.broadcasted_iota(jnp.int32, (RB, LANES), 0)
    even1 = (lane_a & 1) == 0
    even2 = (lane_a & 2) == 0
    scale = DH ** -0.5

    def shifted(ref, r0, i, c, step, n_steps):
        win = after_anchor(ref[pl.ds(r0, RB + HALO), i * LANES:(i + 1) * LANES], step, n_steps)
        lo = HALO - 8 - DIL * c
        blk = win[lo:lo + RB + 8]
        return blk[8:], blk[:RB]

    def attn_block(r0, half):
        logit = [None] * W
        pos = row_a + r0
        for c in range(W // 2):
            ws = (c, c + W // 2)
            for i in range(NT):
                qi = q_v[pl.ds(r0, RB), i * LANES:(i + 1) * LANES]
                for w, kw in zip(ws, shifted(k_v, r0, i, c, i, NT)):
                    logit[w] = qi * kw if i == 0 else logit[w] + qi * kw
            for w in ws:
                s = logit[w]
                s = s + jnp.where(even1, pltpu.roll(s, LANES - 1, 1), pltpu.roll(s, 1, 1))
                s = s + jnp.where(even2, pltpu.roll(s, LANES - 2, 1), pltpu.roll(s, 2, 1))
                s = s * scale
                logit[w] = s if w == 0 else jnp.where(pos >= DIL * w, s, -1e9)
            yield [logit[w] for w in ws]
        m = logit[0]
        for w in range(1, W):
            m = jnp.maximum(m, logit[w])
        e = [jnp.exp(s - m) for s in logit]
        den = e[0]
        for w in range(1, W):
            den = den + e[w]
        inv = 1.0 / den
        prob = [ew * inv for ew in e]
        yield [inv]
        for i in range(NT):
            acc = None
            for c in range(W // 2):
                for w, vw in zip((c, c + W // 2), shifted(v_v, r0, i, c, c, W // 2)):
                    acc = prob[w] * vw if acc is None else acc + prob[w] * vw
            o_v[pl.ds(half, RB // 2), i * LANES:(i + 1) * LANES] = _pack(acc)
            yield [acc]

    def attn_rows(r0, n_blocks):
        for b in range(n_blocks):
            start_row = r0 + b * RB
            if isinstance(r0, int):
                yield from attn_block(start_row, start_row // 2)
            else:
                yield from attn_block(pl.multiple_of(start_row, RB), pl.multiple_of(start_row // 2, RB // 2))

    slots = D // NP * (D // KP)

    def chunk(r):
        return ("mod", r), ("mod", D + r), ("wq", r)

    def chunk_stages(r):
        sc_rows = jnp.broadcast_to(silu_c(), (MOD_ROWS, D))
        for lo in (r, D + r):
            m = jnp.dot(sc_rows, wmod_v[:, lo:lo + MA], preferred_element_type=F32)
            mod_v[:, lo:lo + MA] = m[0:8].astype(BF16).astype(F32)
        cols = slice(r, r + MA)
        h = _pack(x1_v[1, 0:TA, cols] * (1.0 + mod_row(1)[:, cols]) + mod_row(0)[:, cols])
        ha_v[0:TA // 2, cols] = h
        yield []
        yield from permute_stages(0, r, r + MA)

    start(("x", 0), *[name for r in range(0, D, MA) for name in chunk(r)],
          *[("x", s) for s in range(1, n_a)], ("w", 1), ("w", 2), "wo", "mod_b", "wg", "wu", "wd")
    wait(("x", 0))
    x1_v[1, 0:TA, :] = _layernorm(x_v[0:TA, :].astype(F32))
    wait(*chunk(0))
    for _ in chunk_stages(0):
        pass
    for r in range(0, D, MA):
        if r + MA < D:
            wait(*chunk(r + MA))
            side = spread(chunk_stages(r + MA), 1 + MA // PR, D // LANES)
        else:
            wait(("x", 1))
            side = spread(ln_stages(x_v, ha_v, TA, TA, 0, 1), TA // LB, D // LANES)
        nq = 4 * LANES * LANES // MA
        for lo in range(0, D, nq):
            parts = lane_tiles(jnp.dot(pltpu.bitcast(ha_v[0:TA // 2, r:r + MA], BF16),
                                       _load_bf16(wq_v, slice(r, r + MA), slice(lo, lo + nq)),
                                       preferred_element_type=F32))
            for j, part in enumerate(parts):
                cols = slice(lo + j * LANES, lo + (j + 1) * LANES)
                if r > 0:
                    part = q_v[0:TA, cols] + part
                q_v[0:TA, cols] = side.step(part)

    def next_ln(s):
        if s == 2:
            wait(("x", 2), ("x", 3))
        yield from ln_stages(x_v, ha_v, s * TA, TA, 0, 1)

    for s in range(1, n_a - 1):
        project(0, s, spread(next_ln(s + 1), TA // LB, slots))
    wait(("w", 1), ("w", 2))
    project(0, n_a - 1, spread(permute_stages(1), D // PR, slots))
    project(1, 0, spread(permute_stages(2), D // PR, slots))
    wait("wo", "mod_b")
    project(2, 0, spread(wo_stages(), NT, slots))
    k_v[0:HALO, :] = jnp.broadcast_to(k_v[HALO:HALO + 1, :], (HALO, D))
    v_v[0:HALO, :] = jnp.broadcast_to(v_v[HALO:HALO + 1, :], (HALO, D))
    attn_stages = TC // RB * ATTN_STAGES
    rest = [(p, s) for s in range(1, n_a) for p in (1, 2)][:-1]
    n_mod = MT * slots
    side = (spread(mod_b_stages(), 4 * D // LANES, n_mod),
            spread(attn_rows(0, TC // RB), attn_stages, len(rest) * slots - n_mod))
    for n, (p, s) in enumerate(rest):
        project(p, s, side[n >= MT])

    def tile_rows(t, n):
        return slice(t * n, (t + 1) * n) if isinstance(t, int) else pl.ds(pl.multiple_of(t * n, n), n)

    def out_proj(t):
        for n, lo in enumerate(range(0, D, NP)):
            cols = slice(lo, lo + NP)
            a = matmul_piece(o_v.at[tile_rows(t, TC // 2)], wo_v, lo, (accg_v, accu_v)[n % 2], None)
            x1_v[t % 2, 0:TC, cols] = x_v[tile_rows(t, TC), cols].astype(F32) + mod_row(2)[:, cols] * a

    def ffn_norm(t, n_slots):
        return spread(ln_stages(x1_v.at[t % 2], h_v, 0, TC, 3, 4), TC // LB, n_slots)

    def out_copy(t, part):
        cols = pl.ds(part * OC, OC)
        return pltpu.make_async_copy(out_v.at[t % 2, :, cols], out_hbm.at[tile_rows(t, TC), cols],
                                     out_sems.at[t % 2, part])

    def out_wait(t):
        for part in range(D // OC):
            out_copy(t, part).wait()

    n_c = S // TC
    n_f = F // NP
    rounds = 2 * (D // KP)

    def down_piece(t, n, side):
        cols = slice(n * NP, (n + 1) * NP)
        y = matmul_piece(act_v, wd_v, n * NP, (accg_v, accu_v)[n % 2], side)
        out_v[t % 2, :, cols] = (x1_v[t % 2, 0:TC, cols] + mod_row(5)[:, cols] * y).astype(BF16)
        if cols.stop % OC == 0:
            out_copy(t, cols.start // OC).start()

    def phase_c(t, carry):
        @pl.when(t >= 2)
        def _():
            out_wait(t - 2)

        nxt = jnp.minimum(t + 1, n_c - 1)
        attn = spread(attn_rows(nxt * TC, TC // RB), attn_stages, n_f * rounds + DW * ND1 * pl.cdiv(F, KP))
        for lo in range(0, F, NP):
            accg_v[...] = matmul_piece(h_v, wg_v, lo, accg_v, attn)
            u = matmul_piece(h_v, wu_v, lo, accu_v, attn)
            act_v[:, lo:lo + NP] = _pack(_silu(accg_v[...]) * u)
        for n in range(ND1):
            down_piece(t, n, (attn,) * DW)

        @pl.when(t < n_c - 1)
        def _():
            out_proj(t + 1)

        norm = ffn_norm(t + 1, (D // NP - ND1) * pl.cdiv(F, KP))
        for n in range(ND1, D // NP):
            down_piece(t, n, norm)
        return carry

    out_proj(0)
    project(2, n_a - 1, ffn_norm(0, slots))
    wait("wg", "wu", "wd")
    lax.fori_loop(0, n_c, phase_c, 0)
    out_wait(n_c - 2)
    out_wait(n_c - 1)


@jax.jit
def pallas_adaLN_cond__sliding_local_dilated__swiglu_ffn__prompt_kernel(
    A_x: jax.Array,
    A_wqkv: jax.Array,
    A_wo: jax.Array,
    B_x: jax.Array,
    B_w_gate: jax.Array,
    B_w_up: jax.Array,
    B_w_down: jax.Array,
    c: jax.Array,
    w_mod: jax.Array,
):
    del B_x
    hbm = pl.BlockSpec(memory_space=pl.ANY)
    out = pl.pallas_call(
        _kernel,
        out_shape=jax.ShapeDtypeStruct((S, D), BF16),
        in_specs=[hbm, hbm, hbm, hbm, hbm, hbm, pl.BlockSpec(memory_space=pltpu.VMEM), hbm,
                  pl.BlockSpec(memory_space=pltpu.SMEM)],
        out_specs=hbm,
        scratch_shapes=[
            pltpu.VMEM((S, D), BF16),
            pltpu.VMEM((3, D, D), BF16),
            pltpu.VMEM((D // 2, D), U32),
            pltpu.VMEM((D // 2, D), U32),
            pltpu.VMEM((D // 2, D), U32),
            pltpu.VMEM((D, D), BF16),
            pltpu.VMEM((D // 2, D), U32),
            pltpu.VMEM((D, F), BF16),
            pltpu.VMEM((D, F), BF16),
            pltpu.VMEM((F, D), BF16),
            pltpu.VMEM((D, 6 * D), BF16),
            pltpu.VMEM((D, LANES), F32),
            pltpu.VMEM((8, 6 * D), F32),
            pltpu.VMEM((S, D), F32),
            pltpu.VMEM((S + HALO, D), F32),
            pltpu.VMEM((S + HALO, D), F32),
            pltpu.VMEM((S // 2, D), U32),
            pltpu.VMEM((TC // 2, F), U32),
            pltpu.VMEM((S // 2, D), U32),
            pltpu.VMEM((TC // 2, D), U32),
            pltpu.VMEM((2, max(TA, TC), D), F32),
            pltpu.VMEM((max(TA, TC), NP), F32),
            pltpu.VMEM((max(TA, TC), NP), F32),
            pltpu.VMEM((2, TC, D), BF16),
            pltpu.SemaphoreType.DMA((7 + S // TA + 3 * D // MA,)),
            pltpu.SemaphoreType.DMA((2, D // OC)),
        ],
        compiler_params=pltpu.CompilerParams(vmem_limit_bytes=120 * 1024 * 1024),
    )(A_x.reshape(S, D), A_wqkv, A_wo, B_w_gate, B_w_up, B_w_down, c, w_mod, jnp.zeros((1,), jnp.int32))
    return out.reshape(1, S, D)
```

```python
import jax
import jax.numpy as jnp
from jax import lax
from jax.experimental import pallas as pl
from jax.experimental.pallas import tpu as pltpu

S, D, F = 2048, 1024, 3584
H, DH, W, DIL = 32, 32, 8, 2
LANES = 128
NT = D // LANES
HALO = 16
TA = 512
RB = 32
TC = 512
NP, KP = 256, 512
PR = 64
LB = 64
MOD_ROWS, MA, MB = 16, 128, 32
OC = 256
ND1, DW = 3, 2
MT = 1
EPS = 1e-5
assert TA == TC
F32, BF16, U32 = jnp.float32, jnp.bfloat16, jnp.uint32


def _layernorm(x):
    m = jnp.mean(x, axis=-1, keepdims=True)
    xc = x - m
    v = jnp.mean(xc * xc, axis=-1, keepdims=True)
    return xc * lax.rsqrt(v + EPS)


def _silu(x):
    half = 0.5 * x
    return half + half * jnp.tanh(half)


ATTN_STAGES = W // 2 + 1 + NT


class _Spread:
    def __init__(self, gen, n_stages, n_slots, never, anchor):
        self.gen, self.n_stages, self.n_slots = gen, n_stages, n_slots
        self.never, self.anchor = never, anchor
        self.slot = self.done = 0
        self.pending = []

    def step(self, part):
        part, rest = part[:, :LANES], part[:, LANES:] if part.shape[1] > LANES else None
        if self.pending:
            tied = jnp.concatenate(self.pending, axis=0)
            for lo in range(0, tied.shape[0], part.shape[0]):
                n = min(part.shape[0], tied.shape[0] - lo)
                tail = jnp.where(self.never, tied[lo:lo + n], part[-n:])
                part = tail if n == part.shape[0] else jnp.concatenate([part[:-n], tail], axis=0)
        self.pending = []
        self.slot += 1
        while self.done < min(self.n_stages, self.n_stages * self.slot // (self.n_slots - 1)):
            self.anchor.append(part)
            self.pending += next(self.gen)
            self.anchor.pop()
            self.done += 1
        return part if rest is None else jnp.concatenate([part, rest], axis=1)


def _pack(x):
    return pltpu.bitcast(x.astype(BF16), U32)


def _load_bf16(ref, rows, cols):
    if ref.dtype == BF16:
        return ref[rows, cols]
    return pltpu.bitcast(ref[rows.start // 2:rows.stop // 2, cols], BF16)


def _kernel(x_hbm, wqkv_hbm, wo_hbm, wg_hbm, wu_hbm, wd_hbm, c_ref, wmod_hbm, zero_ref, out_hbm,
            x_v, wqkv_raw, wq_v, wk_v, wv_v, wo_raw, wo_v, wg_v, wu_v, wd_v, wmod_v, sc_v, mod_v,
            q_v, k_v, v_v, o_v, act_v, ha_v, h_v, x1_v, accg_v, accu_v, out_v, sems, out_sems):
    n_a = S // TA
    copies = {}

    def add_copy(name, src, dst):
        copies[name] = pltpu.make_async_copy(src, dst, sems.at[len(copies)])

    for r in range(0, D, MA):
        add_copy(("wq", r), wqkv_hbm.at[pl.ds(r, MA), pl.ds(0, D)], wqkv_raw.at[0, pl.ds(r, MA)])
    for p in (1, 2):
        add_copy(("w", p), wqkv_hbm.at[:, pl.ds(p * D, D)], wqkv_raw.at[p])
    for s in range(n_a):
        add_copy(("x", s), x_hbm.at[pl.ds(s * TA, TA)], x_v.at[pl.ds(s * TA, TA)])
    for lo in range(0, 2 * D, MA):
        add_copy(("mod", lo), wmod_hbm.at[:, pl.ds(lo, MA)], wmod_v.at[:, pl.ds(lo, MA)])
    add_copy("mod_b", wmod_hbm.at[:, pl.ds(2 * D, 4 * D)], wmod_v.at[:, pl.ds(2 * D, 4 * D)])
    add_copy("wo", wo_hbm, wo_raw)
    add_copy("wg", wg_hbm, wg_v)
    add_copy("wu", wu_hbm, wu_v)
    add_copy("wd", wd_hbm, wd_v)

    def start(*names):
        for name in names:
            copies[name].start()

    def wait(*names):
        for name in names:
            copies[name].wait()

    never = lax.broadcasted_iota(jnp.int32, (1, LANES), 1) < zero_ref[0]
    anchor = []

    def spread(gen, n_stages, n_slots):
        return _Spread(gen, n_stages, n_slots, never, anchor)

    def after_anchor(x, i=0, n=1):
        if not anchor:
            return x
        lo = min(anchor[-1].shape[0] * i // n, anchor[-1].shape[0] - x.shape[0])
        a = anchor[-1][lo:lo + x.shape[0]]
        return jnp.concatenate([jnp.where(never, a, x[:, j:j + LANES]) for j in range(0, x.shape[1], LANES)], axis=1)

    def silu_c():
        return _silu(c_ref[...].astype(F32)).astype(BF16)

    def mod_row(i):
        return mod_v[0:1, i * D:(i + 1) * D]

    def mod_b_stages():
        sc = silu_c().astype(F32)
        for lo in range(0, D, LANES):
            sc_v[lo:lo + LANES, :] = jnp.broadcast_to(sc[:, lo:lo + LANES], (LANES, LANES)).T
        for lo in range(2 * D, 6 * D, LANES):
            acc = None
            for r in range(0, D, MB):
                part = wmod_v[r:r + MB, lo:lo + LANES].astype(F32) * sc_v[r:r + MB, :]
                if r % (4 * MB) == 0:
                    part = after_anchor(part, r, D)
                acc = part if acc is None else acc + part
            row = jnp.sum(acc, axis=0, keepdims=True).astype(BF16).astype(F32)
            row = jnp.broadcast_to(row, (8, LANES))
            mod_v[:, lo:lo + LANES] = row
            yield [row]

    def lane_tiles(v):
        return [v[:, j * LANES:(j + 1) * LANES] for j in range(v.shape[1] // LANES)]

    def ln_stages(src, dst, r0, n_rows, shift, scale):
        for r in range(r0, r0 + n_rows, LB):
            x = src[r:r + LB, :].astype(F32)
            x = jnp.concatenate([after_anchor(x[:, :LANES], r // LB % 2, 2), x[:, LANES:]], axis=1)
            h = _layernorm(x) * (1.0 + mod_row(scale)) + mod_row(shift)
            h = _pack(h)
            dst[r // 2:(r + LB) // 2, :] = h
            yield [pltpu.bitcast(t, F32) for t in lane_tiles(h)]

    def permute_rows_of(p, r):
        lane = lax.broadcasted_iota(jnp.int32, (PR // 2, LANES), 1)
        t = [_pack(wqkv_raw[p, pl.ds(2 * r, PR), j * LANES:(j + 1) * LANES]) for j in range(NT)]
        t[0] = pltpu.bitcast(after_anchor(pltpu.bitcast(t[0], F32)), U32)
        for b in range(3):
            sh = 4 << b
            low = (lane & sh) == 0
            for j in range(NT):
                if j & (1 << b):
                    continue
                lo_t, hi_t = t[j], t[j | (1 << b)]
                t[j] = jnp.where(low, lo_t, pltpu.roll(hi_t, sh, 1))
                t[j | (1 << b)] = jnp.where(low, pltpu.roll(lo_t, LANES - sh, 1), hi_t)
        for j in range(NT):
            (wq_v, wk_v, wv_v)[p][pl.ds(r, PR // 2), j * LANES:(j + 1) * LANES] = t[j]
        return [pltpu.bitcast(tj, F32) for tj in t]

    def permute_stages(p, lo=0, hi=D):
        for r in range(lo // 2, hi // 2, PR // 2):
            yield permute_rows_of(p, r)

    def wo_stages():
        for i in range(NT):
            done = []
            for hh in range(4):
                for jq in range(NT // 4):
                    pieces = []
                    for j in range(4 * jq, 4 * jq + 4):
                        src = (4 * j + hh) * DH + 4 * i
                        grp = wo_raw[src // 16 * 16:src // 16 * 16 + 16, :].astype(F32)
                        pieces.append(grp[src % 16:src % 16 + 4])
                    dst = i * LANES + hh * DH + jq * 16
                    blk = _pack(jnp.concatenate(pieces, axis=0))
                    wo_v[dst // 2:dst // 2 + 8, :] = blk
                    done += [pltpu.bitcast(t, F32) for t in lane_tiles(blk)]
            yield done

    def matmul_piece(lhs_ref, w_ref, lo, acc_ref, side):
        n_k = pl.cdiv(lhs_ref.shape[1], KP)
        for i in range(n_k):
            ks = slice(i * KP, min((i + 1) * KP, lhs_ref.shape[1]))
            part = jnp.dot(pltpu.bitcast(lhs_ref[:, ks], BF16), _load_bf16(w_ref, ks, slice(lo, lo + NP)),
                           preferred_element_type=F32)
            if i > 0:
                part = acc_ref[...] + part
            for sd in (side if isinstance(side, tuple) else () if side is None else (side,)):
                part = sd.step(part)
            if i == n_k - 1:
                return part
            acc_ref[...] = part

    def project(p, s, side=None):
        dst, off = ((q_v, 0), (k_v, HALO), (v_v, HALO))[p]
        r0 = s * TA
        for n, lo in enumerate(range(0, D, NP)):
            acc = (accg_v, accu_v)[n % 2].at[0:TA]
            dst[r0 + off:r0 + off + TA, lo:lo + NP] = matmul_piece(
                ha_v.at[r0 // 2:(r0 + TA) // 2], (wq_v, wk_v, wv_v)[p], lo, acc, side)

    lane_a = lax.broadcasted_iota(jnp.int32, (RB, LANES), 1)
    row_a = lax.broadcasted_iota(jnp.int32, (RB, LANES), 0)
    even1 = (lane_a & 1) == 0
    even2 = (lane_a & 2) == 0
    scale = DH ** -0.5

    def shifted(ref, r0, i, c, step, n_steps):
        win = after_anchor(ref[pl.ds(r0, RB + HALO), i * LANES:(i + 1) * LANES], step, n_steps)
        lo = HALO - 8 - DIL * c
        blk = win[lo:lo + RB + 8]
        return blk[8:], blk[:RB]

    def attn_block(r0, half):
        logit = [None] * W
        pos = row_a + r0
        for c in range(W // 2):
            ws = (c, c + W // 2)
            for i in range(NT):
                qi = q_v[pl.ds(r0, RB), i * LANES:(i + 1) * LANES]
                for w, kw in zip(ws, shifted(k_v, r0, i, c, i, NT)):
                    logit[w] = qi * kw if i == 0 else logit[w] + qi * kw
            for w in ws:
                s = logit[w]
                s = s + jnp.where(even1, pltpu.roll(s, LANES - 1, 1), pltpu.roll(s, 1, 1))
                s = s + jnp.where(even2, pltpu.roll(s, LANES - 2, 1), pltpu.roll(s, 2, 1))
                s = s * scale
                logit[w] = s if w == 0 else jnp.where(pos >= DIL * w, s, -1e9)
            yield [logit[w] for w in ws]
        m = logit[0]
        for w in range(1, W):
            m = jnp.maximum(m, logit[w])
        e = [jnp.exp(s - m) for s in logit]
        den = e[0]
        for w in range(1, W):
            den = den + e[w]
        inv = 1.0 / den
        prob = [ew * inv for ew in e]
        yield [inv]
        for i in range(NT):
            acc = None
            for c in range(W // 2):
                for w, vw in zip((c, c + W // 2), shifted(v_v, r0, i, c, c, W // 2)):
                    acc = prob[w] * vw if acc is None else acc + prob[w] * vw
            o_v[pl.ds(half, RB // 2), i * LANES:(i + 1) * LANES] = _pack(acc)
            yield [acc]

    def attn_rows(r0, n_blocks):
        for b in range(n_blocks):
            start_row = r0 + b * RB
            if isinstance(r0, int):
                yield from attn_block(start_row, start_row // 2)
            else:
                yield from attn_block(pl.multiple_of(start_row, RB), pl.multiple_of(start_row // 2, RB // 2))

    slots = D // NP * (D // KP)

    def chunk(r):
        return ("mod", r), ("mod", D + r), ("wq", r)

    def chunk_stages(r):
        sc_rows = jnp.broadcast_to(silu_c(), (MOD_ROWS, D))
        for lo in (r, D + r):
            m = jnp.dot(sc_rows, wmod_v[:, lo:lo + MA], preferred_element_type=F32)
            mod_v[:, lo:lo + MA] = m[0:8].astype(BF16).astype(F32)
        cols = slice(r, r + MA)
        h = _pack(x1_v[1, 0:TA, cols] * (1.0 + mod_row(1)[:, cols]) + mod_row(0)[:, cols])
        ha_v[0:TA // 2, cols] = h
        yield []
        yield from permute_stages(0, r, r + MA)

    start(("x", 0), *[name for r in range(0, D, MA) for name in chunk(r)],
          *[("x", s) for s in range(1, n_a)], ("w", 1), ("w", 2), "wo", "mod_b", "wg", "wu", "wd")
    wait(("x", 0))
    x1_v[1, 0:TA, :] = _layernorm(x_v[0:TA, :].astype(F32))
    wait(*chunk(0))
    for _ in chunk_stages(0):
        pass
    for r in range(0, D, MA):
        if r + MA < D:
            wait(*chunk(r + MA))
            side = spread(chunk_stages(r + MA), 1 + MA // PR, D // LANES)
        else:
            wait(("x", 1))
            side = spread(ln_stages(x_v, ha_v, TA, TA, 0, 1), TA // LB, D // LANES)
        nq = 4 * LANES * LANES // MA
        for lo in range(0, D, nq):
            parts = lane_tiles(jnp.dot(pltpu.bitcast(ha_v[0:TA // 2, r:r + MA], BF16),
                                       _load_bf16(wq_v, slice(r, r + MA), slice(lo, lo + nq)),
                                       preferred_element_type=F32))
            for j, part in enumerate(parts):
                cols = slice(lo + j * LANES, lo + (j + 1) * LANES)
                if r > 0:
                    part = q_v[0:TA, cols] + part
                q_v[0:TA, cols] = side.step(part)

    def next_ln(s):
        if s == 2:
            wait(("x", 2), ("x", 3))
        yield from ln_stages(x_v, ha_v, s * TA, TA, 0, 1)

    for s in range(1, n_a - 1):
        project(0, s, spread(next_ln(s + 1), TA // LB, slots))
    wait(("w", 1), ("w", 2))
    project(0, n_a - 1, spread(permute_stages(1), D // PR, slots))
    project(1, 0, spread(permute_stages(2), D // PR, slots))
    wait("wo", "mod_b")
    project(2, 0, spread(wo_stages(), NT, slots))
    k_v[0:HALO, :] = jnp.broadcast_to(k_v[HALO:HALO + 1, :], (HALO, D))
    v_v[0:HALO, :] = jnp.broadcast_to(v_v[HALO:HALO + 1, :], (HALO, D))
    attn_stages = TC // RB * ATTN_STAGES
    rest = [(p, s) for s in range(1, n_a) for p in (1, 2)][:-1]
    n_mod = MT * slots
    side = (spread(mod_b_stages(), 4 * D // LANES, n_mod),
            spread(attn_rows(0, TC // RB), attn_stages, len(rest) * slots - n_mod))
    for n, (p, s) in enumerate(rest):
        project(p, s, side[n >= MT])

    def tile_rows(t, n):
        return slice(t * n, (t + 1) * n) if isinstance(t, int) else pl.ds(pl.multiple_of(t * n, n), n)

    def out_proj(t):
        for n, lo in enumerate(range(0, D, NP)):
            cols = slice(lo, lo + NP)
            a = matmul_piece(o_v.at[tile_rows(t, TC // 2)], wo_v, lo, (accg_v, accu_v)[n % 2], None)
            x1_v[t % 2, 0:TC, cols] = x_v[tile_rows(t, TC), cols].astype(F32) + mod_row(2)[:, cols] * a

    def ffn_norm(t, n_slots):
        return spread(ln_stages(x1_v.at[t % 2], h_v, 0, TC, 3, 4), TC // LB, n_slots)

    def out_copy(t, part):
        cols = pl.ds(part * OC, OC)
        return pltpu.make_async_copy(out_v.at[t % 2, :, cols], out_hbm.at[tile_rows(t, TC), cols],
                                     out_sems.at[t % 2, part])

    def out_wait(t):
        for part in range(D // OC):
            out_copy(t, part).wait()

    n_c = S // TC
    n_f = F // NP
    rounds = 2 * (D // KP)

    def down_piece(t, n, side):
        cols = slice(n * NP, (n + 1) * NP)
        y = matmul_piece(act_v, wd_v, n * NP, (accg_v, accu_v)[n % 2], side)
        out_v[t % 2, :, cols] = (x1_v[t % 2, 0:TC, cols] + mod_row(5)[:, cols] * y).astype(BF16)
        if cols.stop % OC == 0:
            out_copy(t, cols.start // OC).start()

    def phase_c(t, carry):
        @pl.when(t >= 2)
        def _():
            out_wait(t - 2)

        nxt = jnp.minimum(t + 1, n_c - 1)
        attn = spread(attn_rows(nxt * TC, TC // RB), attn_stages, n_f * rounds + DW * ND1 * pl.cdiv(F, KP))
        for lo in range(0, F, NP):
            accg_v[...] = matmul_piece(h_v, wg_v, lo, accg_v, attn)
            u = matmul_piece(h_v, wu_v, lo, accu_v, attn)
            act_v[:, lo:lo + NP] = _pack(_silu(accg_v[...]) * u)
        for n in range(ND1):
            down_piece(t, n, (attn,) * DW)

        @pl.when(t < n_c - 1)
        def _():
            out_proj(t + 1)

        norm = ffn_norm(t + 1, (D // NP - ND1) * pl.cdiv(F, KP))
        for n in range(ND1, D // NP):
            down_piece(t, n, norm)
        return carry

    out_proj(0)
    project(2, n_a - 1, ffn_norm(0, slots))
    wait("wg", "wu", "wd")
    lax.fori_loop(0, n_c, phase_c, 0)
    out_wait(n_c - 2)
    out_wait(n_c - 1)


@jax.jit
def pallas_adaLN_cond__sliding_local_dilated__swiglu_ffn__prompt_kernel(
    A_x: jax.Array,
    A_wqkv: jax.Array,
    A_wo: jax.Array,
    B_x: jax.Array,
    B_w_gate: jax.Array,
    B_w_up: jax.Array,
    B_w_down: jax.Array,
    c: jax.Array,
    w_mod: jax.Array,
):
    del B_x
    hbm = pl.BlockSpec(memory_space=pl.ANY)
    out = pl.pallas_call(
        _kernel,
        out_shape=jax.ShapeDtypeStruct((S, D), BF16),
        in_specs=[hbm, hbm, hbm, hbm, hbm, hbm, pl.BlockSpec(memory_space=pltpu.VMEM), hbm,
                  pl.BlockSpec(memory_space=pltpu.SMEM)],
        out_specs=hbm,
        scratch_shapes=[
            pltpu.VMEM((S, D), BF16),
            pltpu.VMEM((3, D, D), BF16),
            pltpu.VMEM((D // 2, D), U32),
            pltpu.VMEM((D // 2, D), U32),
            pltpu.VMEM((D // 2, D), U32),
            pltpu.VMEM((D, D), BF16),
            pltpu.VMEM((D // 2, D), U32),
            pltpu.VMEM((D, F), BF16),
            pltpu.VMEM((D, F), BF16),
            pltpu.VMEM((F, D), BF16),
            pltpu.VMEM((D, 6 * D), BF16),
            pltpu.VMEM((D, LANES), F32),
            pltpu.VMEM((8, 6 * D), F32),
            pltpu.VMEM((S, D), F32),
            pltpu.VMEM((S + HALO, D), F32),
            pltpu.VMEM((S + HALO, D), F32),
            pltpu.VMEM((S // 2, D), U32),
            pltpu.VMEM((TC // 2, F), U32),
            pltpu.VMEM((S // 2, D), U32),
            pltpu.VMEM((TC // 2, D), U32),
            pltpu.VMEM((2, max(TA, TC), D), F32),
            pltpu.VMEM((max(TA, TC), NP), F32),
            pltpu.VMEM((max(TA, TC), NP), F32),
            pltpu.VMEM((2, TC, D), BF16),
            pltpu.SemaphoreType.DMA((7 + S // TA + 3 * D // MA,)),
            pltpu.SemaphoreType.DMA((2, D // OC)),
        ],
        compiler_params=pltpu.CompilerParams(vmem_limit_bytes=120 * 1024 * 1024),
    )(A_x.reshape(S, D), A_wqkv, A_wo, B_w_gate, B_w_up, B_w_down, c, w_mod, jnp.zeros((1,), jnp.int32))
    return out.reshape(1, S, D)
```

```python
import jax
import jax.numpy as jnp
import numpy as np
from jax import lax
from jax.experimental import pallas as pl
from jax.experimental.pallas import tpu as pltpu

S, D, F = 2048, 1024, 3584
H, DH, W, DIL = 32, 32, 8, 2
LANES = 128
NT = D // LANES
HALO = 16
TA = 512
RB = 32
TC = 512
NP, KP = 256, 512
PR = 64
LB = 64
MOD_ROWS, MA, MB = 16, 128, 32
OC = 256
ND1, DW = 3, 2
MT = 1
EPS = 1e-5
assert TA == TC
F32, BF16, U32 = jnp.float32, jnp.bfloat16, jnp.uint32


def _layernorm(x):
    m = jnp.mean(x, axis=-1, keepdims=True)
    xc = x - m
    v = jnp.mean(xc * xc, axis=-1, keepdims=True)
    return xc * lax.rsqrt(v + EPS)


def _silu(x):
    half = 0.5 * x
    return half + half * jnp.tanh(half)


ATTN_STAGES = W // 2 + 1 + NT


class _Spread:
    def __init__(self, gen, n_stages, n_slots, never, anchor):
        self.gen, self.n_stages, self.n_slots = gen, n_stages, n_slots
        self.never, self.anchor = never, anchor
        self.slot = self.done = 0
        self.pending = []

    def step(self, part):
        part, rest = part[:, :LANES], part[:, LANES:] if part.shape[1] > LANES else None
        if self.pending:
            tied = jnp.concatenate(self.pending, axis=0)
            for lo in range(0, tied.shape[0], part.shape[0]):
                n = min(part.shape[0], tied.shape[0] - lo)
                tail = jnp.where(self.never, tied[lo:lo + n], part[-n:])
                part = tail if n == part.shape[0] else jnp.concatenate([part[:-n], tail], axis=0)
        self.pending = []
        self.slot += 1
        while self.done < min(self.n_stages, self.n_stages * self.slot // (self.n_slots - 1)):
            self.anchor.append(part)
            self.pending += next(self.gen)
            self.anchor.pop()
            self.done += 1
        return part if rest is None else jnp.concatenate([part, rest], axis=1)


def _pack(x):
    return pltpu.bitcast(x.astype(BF16), U32)


def _load_bf16(ref, rows, cols):
    if ref.dtype == BF16:
        return ref[rows, cols]
    return pltpu.bitcast(ref[rows.start // 2:rows.stop // 2, cols], BF16)


def _kernel(x_hbm, wqkv_hbm, wo_hbm, wg_hbm, wu_hbm, wd_hbm, c_ref, wmod_hbm, zero_ref, out_hbm,
            x_v, wqkv_raw, wq_v, wk_v, wv_v, wo_raw, wo_v, wg_v, wu_v, wd_v, wmod_v, sc_v, mod_v,
            q_v, k_v, v_v, o_v, act_v, ha_v, h_v, x1_v, accg_v, accu_v, out_v, sems, out_sems):
    n_a = S // TA
    copies = {}

    def add_copy(name, src, dst):
        copies[name] = pltpu.make_async_copy(src, dst, sems.at[len(copies)])

    for r in range(0, D, MA):
        add_copy(("wq", r), wqkv_hbm.at[pl.ds(r, MA), pl.ds(0, D)], wqkv_raw.at[0, pl.ds(r, MA)])
    for p in (1, 2):
        add_copy(("w", p), wqkv_hbm.at[:, pl.ds(p * D, D)], wqkv_raw.at[p])
    for s in range(n_a):
        add_copy(("x", s), x_hbm.at[pl.ds(s * TA, TA)], x_v.at[pl.ds(s * TA, TA)])
    for lo in range(0, 2 * D, MA):
        add_copy(("mod", lo), wmod_hbm.at[:, pl.ds(lo, MA)], wmod_v.at[:, pl.ds(lo, MA)])
    add_copy("mod_b", wmod_hbm.at[:, pl.ds(2 * D, 4 * D)], wmod_v.at[:, pl.ds(2 * D, 4 * D)])
    add_copy("wo", wo_hbm, wo_raw)
    add_copy("wg", wg_hbm, wg_v)
    add_copy("wu", wu_hbm, wu_v)
    add_copy("wd", wd_hbm, wd_v)

    def start(*names):
        for name in names:
            copies[name].start()

    def wait(*names):
        for name in names:
            copies[name].wait()

    never = lax.broadcasted_iota(jnp.int32, (1, LANES), 1) < zero_ref[0]
    anchor = []

    def spread(gen, n_stages, n_slots):
        return _Spread(gen, n_stages, n_slots, never, anchor)

    def after_anchor(x, i=0, n=1):
        if not anchor:
            return x
        lo = min(anchor[-1].shape[0] * i // n, anchor[-1].shape[0] - x.shape[0])
        a = anchor[-1][lo:lo + x.shape[0]]
        return jnp.concatenate([jnp.where(never, a, x[:, j:j + LANES]) for j in range(0, x.shape[1], LANES)], axis=1)

    def silu_c():
        return _silu(c_ref[...].astype(F32)).astype(BF16)

    def mod_row(i, cols=slice(0, D)):
        return mod_v[0:1, i * D + cols.start:i * D + cols.stop]

    def mod_b_stages():
        sc = silu_c().astype(F32)
        for lo in range(0, D, LANES):
            sc_v[lo:lo + LANES, :] = jnp.broadcast_to(sc[:, lo:lo + LANES], (LANES, LANES)).T
        for lo in range(2 * D, 6 * D, LANES):
            acc = None
            for r in range(0, D, MB):
                part = wmod_v[r:r + MB, lo:lo + LANES].astype(F32) * sc_v[r:r + MB, :]
                if r % (4 * MB) == 0:
                    part = after_anchor(part, r, D)
                acc = part if acc is None else acc + part
            row = jnp.sum(acc, axis=0, keepdims=True).astype(BF16).astype(F32)
            row = jnp.broadcast_to(row, (8, LANES))
            mod_v[:, lo:lo + LANES] = row
            yield [row]

    def lane_tiles(v):
        return [v[:, j * LANES:(j + 1) * LANES] for j in range(v.shape[1] // LANES)]

    def ln_stages(src, dst, r0, n_rows, shift, scale):
        for r in range(r0, r0 + n_rows, LB):
            x = src[r:r + LB, :].astype(F32)
            x = jnp.concatenate([after_anchor(x[:, :LANES], r // LB % 2, 2), x[:, LANES:]], axis=1)
            h = _layernorm(x) * (1.0 + mod_row(scale)) + mod_row(shift)
            h = _pack(h)
            dst[r // 2:(r + LB) // 2, :] = h
            yield [pltpu.bitcast(t, F32) for t in lane_tiles(h)]

    def permute_rows_of(p, r):
        lane = lax.broadcasted_iota(jnp.int32, (PR // 2, LANES), 1)
        t = [_pack(wqkv_raw[p, pl.ds(2 * r, PR), j * LANES:(j + 1) * LANES]) for j in range(NT)]
        t[0] = pltpu.bitcast(after_anchor(pltpu.bitcast(t[0], F32)), U32)
        for b in range(3):
            sh = 4 << b
            low = (lane & sh) == 0
            for j in range(NT):
                if j & (1 << b):
                    continue
                lo_t, hi_t = t[j], t[j | (1 << b)]
                t[j] = jnp.where(low, lo_t, pltpu.roll(hi_t, sh, 1))
                t[j | (1 << b)] = jnp.where(low, pltpu.roll(lo_t, LANES - sh, 1), hi_t)
        for j in range(NT):
            (wq_v, wk_v, wv_v)[p][pl.ds(r, PR // 2), j * LANES:(j + 1) * LANES] = t[j]
        return [pltpu.bitcast(tj, F32) for tj in t]

    def permute_stages(p, lo=0, hi=D):
        for r in range(lo // 2, hi // 2, PR // 2):
            yield permute_rows_of(p, r)

    def wo_stages():
        for i in range(NT):
            done = []
            for hh in range(4):
                for jq in range(NT // 4):
                    pieces = []
                    for j in range(4 * jq, 4 * jq + 4):
                        src = (4 * j + hh) * DH + 4 * i
                        grp = wo_raw[src // 16 * 16:src // 16 * 16 + 16, :].astype(F32)
                        pieces.append(grp[src % 16:src % 16 + 4])
                    dst = i * LANES + hh * DH + jq * 16
                    blk = _pack(jnp.concatenate(pieces, axis=0))
                    wo_v[dst // 2:dst // 2 + 8, :] = blk
                    done += [pltpu.bitcast(t, F32) for t in lane_tiles(blk)]
            yield done

    def matmul_piece(lhs_ref, w_ref, lo, acc_ref, side):
        n_k = pl.cdiv(lhs_ref.shape[1], KP)
        for i in range(n_k):
            ks = slice(i * KP, min((i + 1) * KP, lhs_ref.shape[1]))
            part = jnp.dot(pltpu.bitcast(lhs_ref[:, ks], BF16), _load_bf16(w_ref, ks, slice(lo, lo + NP)),
                           preferred_element_type=F32)
            if i > 0:
                part = acc_ref[...] + part
            for sd in (side if isinstance(side, tuple) else () if side is None else (side,)):
                part = sd.step(part)
            if i == n_k - 1:
                return part
            acc_ref[...] = part

    def project(p, s, side=None):
        dst, off = ((q_v, 0), (k_v, HALO), (v_v, HALO))[p]
        r0 = s * TA
        for n, lo in enumerate(range(0, D, NP)):
            acc = (accg_v, accu_v)[n % 2].at[0:TA]
            dst[r0 + off:r0 + off + TA, lo:lo + NP] = matmul_piece(
                ha_v.at[r0 // 2:(r0 + TA) // 2], (wq_v, wk_v, wv_v)[p], lo, acc, side)

    lane_a = lax.broadcasted_iota(jnp.int32, (RB, LANES), 1)
    row_a = lax.broadcasted_iota(jnp.int32, (RB, LANES), 0)
    even1 = (lane_a & 1) == 0
    even2 = (lane_a & 2) == 0
    scale = DH ** -0.5

    def shifted(ref, r0, i, c, step, n_steps):
        win = after_anchor(ref[pl.ds(r0, RB + HALO), i * LANES:(i + 1) * LANES], step, n_steps)
        lo = HALO - 8 - DIL * c
        blk = win[lo:lo + RB + 8]
        return blk[8:], blk[:RB]

    def attn_block(r0, half):
        logit = [None] * W
        pos = row_a + r0
        for c in range(W // 2):
            ws = (c, c + W // 2)
            for i in range(NT):
                qi = q_v[pl.ds(r0, RB), i * LANES:(i + 1) * LANES]
                for w, kw in zip(ws, shifted(k_v, r0, i, c, i, NT)):
                    logit[w] = qi * kw if i == 0 else logit[w] + qi * kw
            for w in ws:
                s = logit[w]
                s = s + jnp.where(even1, pltpu.roll(s, LANES - 1, 1), pltpu.roll(s, 1, 1))
                s = s + jnp.where(even2, pltpu.roll(s, LANES - 2, 1), pltpu.roll(s, 2, 1))
                s = s * scale
                logit[w] = s if w == 0 else jnp.where(pos >= DIL * w, s, -1e9)
            yield [logit[w] for w in ws]
        m = logit[0]
        for w in range(1, W):
            m = jnp.maximum(m, logit[w])
        e = [jnp.exp(s - m) for s in logit]
        den = e[0]
        for w in range(1, W):
            den = den + e[w]
        inv = 1.0 / den
        prob = [ew * inv for ew in e]
        yield [inv]
        for i in range(NT):
            acc = None
            for c in range(W // 2):
                for w, vw in zip((c, c + W // 2), shifted(v_v, r0, i, c, c, W // 2)):
                    acc = prob[w] * vw if acc is None else acc + prob[w] * vw
            o_v[pl.ds(half, RB // 2), i * LANES:(i + 1) * LANES] = _pack(acc)
            yield [acc]

    def attn_rows(r0, n_blocks):
        for b in range(n_blocks):
            start_row = r0 + b * RB
            if isinstance(r0, int):
                yield from attn_block(start_row, start_row // 2)
            else:
                yield from attn_block(pl.multiple_of(start_row, RB), pl.multiple_of(start_row // 2, RB // 2))

    slots = D // NP * (D // KP)

    def chunk(r):
        return ("mod", r), ("mod", D + r), ("wq", r)

    def chunk_stages(r):
        sc_rows = jnp.broadcast_to(silu_c(), (MOD_ROWS, D))
        for lo in (r, D + r):
            m = jnp.dot(sc_rows, wmod_v[:, lo:lo + MA], preferred_element_type=F32)
            mod_v[:, lo:lo + MA] = m[0:8].astype(BF16).astype(F32)
        cols = slice(r, r + MA)
        h = _pack(x1_v[1, 0:TA, cols] * (1.0 + mod_row(1, cols)) + mod_row(0, cols))
        ha_v[0:TA // 2, cols] = h
        yield []
        yield from permute_stages(0, r, r + MA)

    start(("x", 0), *[name for r in range(0, D, MA) for name in chunk(r)],
          *[("x", s) for s in range(1, n_a)], ("w", 1), ("w", 2), "wo", "mod_b", "wg", "wu", "wd")
    wait(("x", 0))
    x1_v[1, 0:TA, :] = _layernorm(x_v[0:TA, :].astype(F32))
    wait(*chunk(0))
    for _ in chunk_stages(0):
        pass
    for r in range(0, D, MA):
        if r + MA < D:
            wait(*chunk(r + MA))
            side = spread(chunk_stages(r + MA), 1 + MA // PR, D // LANES)
        else:
            wait(("x", 1))
            side = spread(ln_stages(x_v, ha_v, TA, TA, 0, 1), TA // LB, D // LANES)
        nq = 4 * LANES * LANES // MA
        for lo in range(0, D, nq):
            parts = lane_tiles(jnp.dot(pltpu.bitcast(ha_v[0:TA // 2, r:r + MA], BF16),
                                       _load_bf16(wq_v, slice(r, r + MA), slice(lo, lo + nq)),
                                       preferred_element_type=F32))
            for j, part in enumerate(parts):
                cols = slice(lo + j * LANES, lo + (j + 1) * LANES)
                if r > 0:
                    part = q_v[0:TA, cols] + part
                q_v[0:TA, cols] = side.step(part)

    def next_ln(s):
        if s == 2:
            wait(("x", 2), ("x", 3))
        yield from ln_stages(x_v, ha_v, s * TA, TA, 0, 1)

    for s in range(1, n_a - 1):
        project(0, s, spread(next_ln(s + 1), TA // LB, slots))
    wait(("w", 1), ("w", 2))
    project(0, n_a - 1, spread(permute_stages(1), D // PR, slots))
    project(1, 0, spread(permute_stages(2), D // PR, slots))
    wait("wo", "mod_b")
    project(2, 0, spread(wo_stages(), NT, slots))
    k_v[0:HALO, :] = jnp.broadcast_to(k_v[HALO:HALO + 1, :], (HALO, D))
    v_v[0:HALO, :] = jnp.broadcast_to(v_v[HALO:HALO + 1, :], (HALO, D))
    attn_stages = TC // RB * ATTN_STAGES
    rest = [(p, s) for s in range(1, n_a) for p in (1, 2)][:-1]
    n_mod = MT * slots
    side = (spread(mod_b_stages(), 4 * D // LANES, n_mod),
            spread(attn_rows(0, TC // RB), attn_stages, len(rest) * slots - n_mod))
    for n, (p, s) in enumerate(rest):
        project(p, s, side[n >= MT])

    def tile_rows(t, n):
        return slice(t * n, (t + 1) * n) if isinstance(t, int) else pl.ds(pl.multiple_of(t * n, n), n)

    def out_proj(t):
        for n, lo in enumerate(range(0, D, NP)):
            cols = slice(lo, lo + NP)
            a = matmul_piece(o_v.at[tile_rows(t, TC // 2)], wo_v, lo, (accg_v, accu_v)[n % 2], None)
            x1_v[t % 2, 0:TC, cols] = x_v[tile_rows(t, TC), cols].astype(F32) + mod_row(2, cols) * a

    def ffn_norm(t, n_slots):
        return spread(ln_stages(x1_v.at[t % 2], h_v, 0, TC, 3, 4), TC // LB, n_slots)

    def out_copy(t, part):
        cols = pl.ds(part * OC, OC)
        return pltpu.make_async_copy(out_v.at[t % 2, :, cols], out_hbm.at[tile_rows(t, TC), cols],
                                     out_sems.at[t % 2, part])

    def out_wait(t):
        for part in range(D // OC):
            out_copy(t, part).wait()

    n_c = S // TC
    n_f = F // NP
    rounds = 2 * (D // KP)

    def down_piece(t, n, side):
        cols = slice(n * NP, (n + 1) * NP)
        y = matmul_piece(act_v, wd_v, n * NP, (accg_v, accu_v)[n % 2], side)
        out_v[t % 2, :, cols] = (x1_v[t % 2, 0:TC, cols] + mod_row(5, cols) * y).astype(BF16)
        if cols.stop % OC == 0:
            out_copy(t, cols.start // OC).start()

    def phase_c(t, carry):
        @pl.when(t >= 2)
        def _():
            out_wait(t - 2)

        nxt = jnp.minimum(t + 1, n_c - 1)
        attn = spread(attn_rows(nxt * TC, TC // RB), attn_stages, n_f * rounds + DW * ND1 * pl.cdiv(F, KP))
        for lo in range(0, F, NP):
            accg_v[...] = matmul_piece(h_v, wg_v, lo, accg_v, attn)
            u = matmul_piece(h_v, wu_v, lo, accu_v, attn)
            act_v[:, lo:lo + NP] = _pack(_silu(accg_v[...]) * u)
        for n in range(ND1):
            down_piece(t, n, (attn,) * DW)

        @pl.when(t < n_c - 1)
        def _():
            out_proj(t + 1)

        norm = ffn_norm(t + 1, (D // NP - ND1) * pl.cdiv(F, KP))
        for n in range(ND1, D // NP):
            down_piece(t, n, norm)
        return carry

    out_proj(0)
    project(2, n_a - 1, ffn_norm(0, slots))
    wait("wg", "wu", "wd")
    lax.fori_loop(0, n_c, phase_c, 0)
    out_wait(n_c - 2)
    out_wait(n_c - 1)


@jax.jit
def pallas_adaLN_cond__sliding_local_dilated__swiglu_ffn__prompt_kernel(
    A_x: jax.Array,
    A_wqkv: jax.Array,
    A_wo: jax.Array,
    B_x: jax.Array,
    B_w_gate: jax.Array,
    B_w_up: jax.Array,
    B_w_down: jax.Array,
    c: jax.Array,
    w_mod: jax.Array,
):
    del B_x
    hbm = pl.BlockSpec(memory_space=pl.ANY)
    out = pl.pallas_call(
        _kernel,
        out_shape=jax.ShapeDtypeStruct((S, D), BF16),
        in_specs=[hbm, hbm, hbm, hbm, hbm, hbm, pl.BlockSpec(memory_space=pltpu.VMEM), hbm,
                  pl.BlockSpec(memory_space=pltpu.SMEM)],
        out_specs=hbm,
        scratch_shapes=[
            pltpu.VMEM((S, D), BF16),
            pltpu.VMEM((3, D, D), BF16),
            pltpu.VMEM((D // 2, D), U32),
            pltpu.VMEM((D // 2, D), U32),
            pltpu.VMEM((D // 2, D), U32),
            pltpu.VMEM((D, D), BF16),
            pltpu.VMEM((D // 2, D), U32),
            pltpu.VMEM((D, F), BF16),
            pltpu.VMEM((D, F), BF16),
            pltpu.VMEM((F, D), BF16),
            pltpu.VMEM((D, 6 * D), BF16),
            pltpu.VMEM((D, LANES), F32),
            pltpu.VMEM((8, 6 * D), F32),
            pltpu.VMEM((S, D), F32),
            pltpu.VMEM((S + HALO, D), F32),
            pltpu.VMEM((S + HALO, D), F32),
            pltpu.VMEM((S // 2, D), U32),
            pltpu.VMEM((TC // 2, F), U32),
            pltpu.VMEM((S // 2, D), U32),
            pltpu.VMEM((TC // 2, D), U32),
            pltpu.VMEM((2, max(TA, TC), D), F32),
            pltpu.VMEM((max(TA, TC), NP), F32),
            pltpu.VMEM((max(TA, TC), NP), F32),
            pltpu.VMEM((2, TC, D), BF16),
            pltpu.SemaphoreType.DMA((7 + S // TA + 3 * D // MA,)),
            pltpu.SemaphoreType.DMA((2, D // OC)),
        ],
        compiler_params=pltpu.CompilerParams(vmem_limit_bytes=120 * 1024 * 1024),
    )(A_x.reshape(S, D), A_wqkv, A_wo, B_w_gate, B_w_up, B_w_down, c, w_mod, np.zeros((1,), np.int32))
    return out.reshape(1, S, D)
```
